```python
import os as _os
_os.environ.setdefault("JAX_PLATFORMS", "cpu")
import jax
import jax.numpy as jnp

def _softmax(x, axis=-1):
    return jax.nn.softmax(x, axis=axis)
def _gelu(x):
    return jax.nn.gelu(x, approximate=True)
def _silu(x):
    return jax.nn.silu(x)
def _sigmoid(x):
    return jax.nn.sigmoid(x)
def _layernorm(x, axis=-1, eps=1e-5):
    m = jnp.mean(x, axis=axis, keepdims=True)
    v = jnp.var(x, axis=axis, keepdims=True)
    return (x - m) / jnp.sqrt(v + eps)
def _scatter_add(tgt, idx, src, axis=0):
    return tgt.at[idx].add(src)
def _segment_sum(src, seg, n):
    return jax.ops.segment_sum(src, seg, n)
class _Rng:
    def __init__(self, key):
        self._k = key
    def _next(self):
        self._k, sub = jax.random.split(self._k)
        return sub
    def normal(self, shape):
        return jax.random.normal(self._next(), shape, dtype=jnp.bfloat16)
    def randint(self, lo, hi, shape):
        return jax.random.randint(self._next(), shape, lo, hi, dtype=jnp.int32)
    def uniform(self, shape, lo=0.0, hi=1.0):
        return jax.random.uniform(self._next(), shape, jnp.bfloat16, lo, hi)
    def permutation(self, n):
        return jax.random.permutation(self._next(), n)


kernel_name = 'interleave_layers__sliding_block__mha_block__prompt'

def setup_inputs():
    _rng = _Rng(jax.random.key(int.from_bytes(__import__("os").urandom(4), "little")))
    _w = (lambda a: (lambda t: t.astype(jnp.bfloat16) if jnp.issubdtype(t.dtype, jnp.floating) else t)(jnp.asarray(a)))
    def _A_setup():
        B, S, D = 1, 2048, 512
        return {
            "x": _w((lambda *s: _rng.normal(s) * 0.05)(B, S, D)),
            "wqkv": _w((lambda *s: _rng.normal(s) * 0.05)(D, 3 * D)),
            "wo": _w((lambda *s: _rng.normal(s) * 0.05)(D, D)),
        }
    _A_in = _A_setup()

    def _B_setup():
        B, S, D, H = 1, 2048, 512, 32
        return {
            "x": _w((lambda *s: _rng.normal(s) * 0.05)(B, S, D)),
            "wqkv": _w((lambda *s: _rng.normal(s) * 0.05)(D, 3 * D)),
            "wo": _w((lambda *s: _rng.normal(s) * 0.05)(D, D)),
        }
    _B_in = _B_setup()

    return {
        "A_x": _A_in["x"],
        "A_wqkv": _A_in["wqkv"],
        "A_wo": _A_in["wo"],
        "B_x": _B_in["x"],
        "B_wqkv": _B_in["wqkv"],
        "B_wo": _B_in["wo"],
    }

def reference(A_x, A_wqkv, A_wo, B_x, B_wqkv, B_wo):
    def _A_ref(x, wqkv, wo):
        B, S, D = x.shape
        H = 32; Dh = D // H; W = 256
        qkv = (lambda x, *d: x.transpose(*d))((x @ wqkv).reshape(B, S, 3, H, Dh), 2, 0, 3, 1, 4)
        q, k, v = qkv[0], qkv[1], qkv[2]
        scores = jnp.einsum("bhqd,bhkd->bhqk", q, k) * (Dh ** -0.5)
        idx = jnp.arange(S)
        mask = (idx[:, None] - idx[None, :] >= 0) & (idx[:, None] - idx[None, :] < W)
        scores = jnp.where(mask[None, None], scores, -1e9)
        p = _softmax(scores, axis=-1)
        o = jnp.einsum("bhqk,bhkd->bhqd", p, v)
        return (lambda x, *d: x.transpose(*d))(o, 0, 2, 1, 3).reshape(B, S, D) @ wo

    def _B_ref(x, wqkv, wo):
        B, S, D = x.shape
        H = 32
        Dh = D // H
        qkv = (lambda x, *d: x.transpose(*d))((x @ wqkv).reshape(B, S, 3, H, Dh), 2, 0, 3, 1, 4)
        q, k, v = qkv[0], qkv[1], qkv[2]
        scores = jnp.einsum("bhqd,bhkd->bhqk", q, k) * (Dh ** -0.5)
        p = _softmax(scores, axis=-1)
        o = jnp.einsum("bhqk,bhkd->bhqd", p, v)
        return (lambda x, *d: x.transpose(*d))(o, 0, 2, 1, 3).reshape(B, S, D) @ wo

    x = A_x
    x = x + _A_ref(_layernorm(x, axis=-1), A_wqkv, A_wo)
    x = x + _B_ref(_layernorm(x, axis=-1), B_wqkv, B_wo)
    x = x + _A_ref(_layernorm(x, axis=-1), A_wqkv, A_wo)
    x = x + _B_ref(_layernorm(x, axis=-1), B_wqkv, B_wo)
    return x
```

```python
import math

import jax
import jax.numpy as jnp
from jax import lax
import jax.experimental.pallas as pl
import jax.experimental.pallas.tpu as pltpu

S = 2048
D = 512
H = 32
DH = 16
WIN = 256
EPS = 1e-5

T = 128
NT = S // T
NG = D // T
PAD = WIN
NEG = -1e30
QSCALE = (DH ** -0.5) * math.log2(math.e)
TT = 512
LAG = 2

F32 = jnp.float32
BF16 = jnp.bfloat16


def _dot(a, b):
    return jnp.dot(a, b, preferred_element_type=F32)


def _kernel(x_ref, awqkv_ref, awo_ref, bwqkv_ref, bwo_ref, out_ref,
            xT_ref, wqkvT_ref, woT_ref, qT_ref, k_ref, vT_ref, oT_ref,
            s_ref, m_ref, bias_ref):
    for t in range(S // TT):
        xT_ref[:, t * TT:(t + 1) * TT] = x_ref[t * TT:(t + 1) * TT, :].astype(F32).T
    for li, (wq, wo) in enumerate(((awqkv_ref, awo_ref), (bwqkv_ref, bwo_ref))):
        for j in range(3):
            wqkvT_ref[li, j * D:(j + 1) * D, :] = (
                wq[:, j * D:(j + 1) * D].astype(F32).T.astype(BF16))
        woT_ref[li] = wo[...].astype(F32).T.astype(BF16)
    for g in range(NG):
        k_ref[g, 0:PAD, :] = jnp.zeros((PAD, T), BF16)
    vT_ref[:, 0:PAD] = jnp.zeros((D, PAD), BF16)
    row = lax.broadcasted_iota(jnp.int32, (3 * T, T), 0)
    col = lax.broadcasted_iota(jnp.int32, (3 * T, T), 1)
    band = (row > col) & (row <= col + WIN)
    for v in range(3):
        valid = band & (row >= WIN - v * T)
        bias_ref[v] = jnp.where(valid, 0.0, NEG).astype(F32)

    def proj_in(li):
        def body(t, carry):
            t0 = pl.multiple_of(t * TT, TT)
            x = xT_ref[:, pl.ds(t0, TT)]
            mu = jnp.mean(x, axis=0, keepdims=True)
            xc = x - mu
            var = jnp.mean(xc * xc, axis=0, keepdims=True)
            xn = (xc * lax.rsqrt(var + EPS)).astype(BF16)
            q = _dot(wqkvT_ref[li, 0:D, :], xn)
            qT_ref[:, pl.ds(t0, TT)] = (q * QSCALE).astype(BF16)
            kk = _dot(wqkvT_ref[li, D:2 * D, :], xn).T.astype(BF16)
            for g in range(NG):
                k_ref[g, pl.ds(PAD + t0, TT), :] = kk[:, g * T:(g + 1) * T]
            v = _dot(wqkvT_ref[li, 2 * D:3 * D, :], xn)
            vT_ref[:, pl.ds(PAD + t0, TT)] = v.astype(BF16)
            return carry
        lax.fori_loop(0, S // TT, body, 0)

    def proj_out(li):
        def body(t, carry):
            t0 = pl.multiple_of(t * TT, TT)
            y = _dot(woT_ref[li], oT_ref[:, pl.ds(t0, TT)])
            xT_ref[:, pl.ds(t0, TT)] = xT_ref[:, pl.ds(t0, TT)] + y
            return carry
        lax.fori_loop(0, S // TT, body, 0)

    def attn_block(qk_items, pv_items, nk, slot_of, bias):
        n_items = len(qk_items if qk_items is not None else pv_items)
        lprev = None
        for u in range(n_items):
            sb, srow = slot_of(u)
            if qk_items is not None:
                g1, r1, half, q1, k1 = qk_items[u]
                cols = []
                for j in range(4):
                    hh = 4 * half + j
                    parts = []
                    if hh > 0:
                        parts.append(jnp.zeros((DH * hh, T), BF16))
                    parts.append(qT_ref[pl.ds(r1 + DH * hh, DH), pl.ds(q1, T)])
                    if hh < 7:
                        parts.append(jnp.zeros((DH * (7 - hh), T), BF16))
                    cols.append(jnp.concatenate(parts, axis=0))
                w = jnp.concatenate(cols, axis=1)
                m = None
            if pv_items is not None:
                _, r2, half2, q2, k2 = pv_items[u]
                mprev = m_ref[u]
                acc = [None] * 4
                ls = []

            def expo(c):
                sp = s_ref[sb, srow + c * T:srow + (c + 1) * T, :].reshape(T // 8, 8, 4 * T)
                mp = mprev
                dep = None
                if c >= LAG:
                    dep = ls[c - LAG]
                elif lprev is not None:
                    dep = lprev[c - LAG]
                if dep is not None:
                    mp = jnp.minimum(mprev, jnp.maximum(dep, jnp.inf))
                p = jnp.exp2(sp - mp[None])
                ps = jnp.sum(p, axis=0)
                ls.append(ps if not ls else ls[-1] + ps)
                return p.reshape(T, 4 * T).astype(BF16)

            if pv_items is not None:
                pb = expo(0)
            for c in range(nk):
                if qk_items is not None:
                    s = _dot(k_ref[g1, pl.ds(k1 + c * T, T), :], w)
                    if bias is not None:
                        b = bias[c * T:(c + 1) * T, :]
                        s = s + jnp.concatenate([b] * 4, axis=1)
                    s_ref[sb, srow + c * T:srow + (c + 1) * T, :] = s
                    sm = jnp.max(s.reshape(T // 8, 8, 4 * T), axis=0)
                    m = sm if m is None else jnp.maximum(m, sm)
                if pv_items is not None:
                    pb_next = expo(c + 1) if c + 1 < nk else None
                    for j in range(4):
                        hh = 4 * half2 + j
                        o = _dot(vT_ref[pl.ds(r2 + DH * hh, DH), pl.ds(k2 + c * T, T)],
                                 pb[:, j * T:(j + 1) * T])
                        acc[j] = o if acc[j] is None else acc[j] + o
                    pb = pb_next
            if qk_items is not None:
                m_ref[u] = jnp.broadcast_to(jnp.max(m, axis=0, keepdims=True), (8, 4 * T))
            if pv_items is not None:
                linv = 1.0 / jnp.sum(ls[-1], axis=0, keepdims=True)
                for j in range(4):
                    hh = 4 * half2 + j
                    oT_ref[pl.ds(r2 + DH * hh, DH), pl.ds(q2, T)] = (
                        acc[j] * linv[:, j * T:(j + 1) * T]).astype(BF16)
                lprev = ls

    def attn_full():
        def items(b):
            if isinstance(b, int):
                g, q, r = b // NT, (b % NT) * T, (b // NT) * T
            else:
                g = lax.shift_right_logical(b, 4)
                q = pl.multiple_of(lax.bitwise_and(b, NT - 1) * T, T)
                r = pl.multiple_of(g * T, T)
            return [(g, r, half, q, PAD) for half in range(2)]
        slot = lambda u: (u, 0)
        nb = NG * NT
        attn_block(items(0), None, NT, slot, None)

        def body(b, carry):
            attn_block(items(b + 1), items(b), NT, slot, None)
            return carry
        lax.fori_loop(0, nb - 1, body, 0)
        attn_block(None, items(nb - 1), NT, slot, None)

    def attn_window():
        def items(b):
            q = b * T if isinstance(b, int) else pl.multiple_of(b * T, T)
            return [(g, g * T, half, q, q) for g in range(NG) for half in range(2)]
        slot = lambda u: (u // 4, (u % 4) * 3 * T)
        attn_block(items(0), None, 3, slot, bias_ref.at[0])

        def body(b, carry):
            attn_block(items(b + 1), items(b), 3, slot,
                       bias_ref.at[jnp.minimum(b + 1, 2)])
            return carry
        lax.fori_loop(0, NT - 1, body, 0)
        attn_block(None, items(NT - 1), 3, slot, None)

    def two_layers(_, carry):
        proj_in(0)
        attn_window()
        proj_out(0)
        proj_in(1)
        attn_full()
        proj_out(1)
        return carry
    lax.fori_loop(0, 2, two_layers, 0)

    for t in range(S // TT):
        out_ref[t * TT:(t + 1) * TT, :] = xT_ref[:, t * TT:(t + 1) * TT].T.astype(BF16)


@jax.jit
def pallas_interleave_layers__sliding_block__mha_block__prompt_kernel(
    A_x: jax.Array,
    A_wqkv: jax.Array,
    A_wo: jax.Array,
    B_x: jax.Array,
    B_wqkv: jax.Array,
    B_wo: jax.Array,
):
    del B_x
    x = A_x.reshape(S, D)
    out = pl.pallas_call(
        _kernel,
        out_shape=jax.ShapeDtypeStruct((S, D), A_x.dtype),
        scratch_shapes=[
            pltpu.VMEM((D, S), F32),
            pltpu.VMEM((2, 3 * D, D), BF16),
            pltpu.VMEM((2, D, D), BF16),
            pltpu.VMEM((D, S), BF16),
            pltpu.VMEM((NG, S + PAD, T), BF16),
            pltpu.VMEM((D, S + PAD), BF16),
            pltpu.VMEM((D, S), BF16),
            pltpu.VMEM((2, S, 4 * T), F32),
            pltpu.VMEM((8, 8, 4 * T), F32),
            pltpu.VMEM((3, 3 * T, T), F32),
        ],
        compiler_params=pltpu.CompilerParams(vmem_limit_bytes=100 * 1024 * 1024),
        name="interleave_attn",
    )(x, A_wqkv, A_wo, B_wqkv, B_wo)
    return out.reshape(A_x.shape)
```

```python
import math

import jax
import jax.numpy as jnp
from jax import lax
import jax.experimental.pallas as pl
import jax.experimental.pallas.tpu as pltpu

S = 2048
D = 512
H = 32
DH = 16
WIN = 256
EPS = 1e-5

T = 128
NT = S // T
NG = D // T
PT = WIN // T
NEG = -1e30
QSCALE = (DH ** -0.5) * math.log2(math.e)
TT = 512
LAG = 2
VK = 16
SMAX = 60.0
VMAX = 2.0 ** 50
VMIN = 2.0 ** -40

F32 = jnp.float32
BF16 = jnp.bfloat16
U32 = jnp.uint32


def _dot(a, b):
    return jnp.dot(a, b, preferred_element_type=F32)


def _bf(x):
    return pltpu.bitcast(x, BF16)


def _kernel(x_ref, awqkv_ref, awo_ref, bwqkv_ref, bwo_ref, out_ref,
            xT_ref, wqkvT_ref, woT_ref, qT_ref, k_ref, vT_ref, oT_ref,
            s_ref, m_ref, bias_ref, p_ref, qb_ref, kb0_ref, kb1_ref, st_ref):
    qu = qT_ref.bitcast(U32)
    ku = k_ref.bitcast(U32)
    vu = vT_ref.bitcast(U32)
    pu = p_ref.bitcast(U32)
    kbs = (kb0_ref, kb1_ref)

    for t in range(S // TT):
        xT_ref[:, t * TT:(t + 1) * TT] = x_ref[t * TT:(t + 1) * TT, :].astype(F32).T
    for li, (wq, wo) in enumerate(((awqkv_ref, awo_ref), (bwqkv_ref, bwo_ref))):
        for j in range(3):
            wqkvT_ref[li, j * D:(j + 1) * D, :] = (
                wq[:, j * D:(j + 1) * D].astype(F32).T.astype(BF16))
        woT_ref[li] = wo[...].astype(F32).T.astype(BF16)
    for g in range(NG):
        k_ref[g, 0:WIN, :] = jnp.zeros((WIN, T), BF16)
    for c in range(PT):
        vT_ref[c] = jnp.zeros((D, T), BF16)
    row = lax.broadcasted_iota(jnp.int32, (3 * T, T), 0)
    col = lax.broadcasted_iota(jnp.int32, (3 * T, T), 1)
    band = (row > col) & (row <= col + WIN)
    for v in range(3):
        valid = band & (row >= WIN - v * T)
        bias_ref[v] = jnp.where(valid, 0.0, NEG).astype(F32)

    def build_kb(kb, kk, c, d0, d1):
        cols = []
        for d in range(d0, d1):
            colv = jnp.broadcast_to(kk[:, d:d + 1], (VK, T))
            kb[c, d] = colv
            cols.append(colv)
        return cols

    def head_norm2(a):
        n2 = jnp.sum((a * a).reshape(H, DH, TT), axis=1)
        return jnp.max(n2.reshape(H // 8, 8, TT), axis=0)

    def proj_in(li, full):
        st_ref[...] = jnp.zeros(st_ref.shape, F32)

        def body(t, carry):
            t0 = pl.multiple_of(t * TT, TT)
            x = xT_ref[:, pl.ds(t0, TT)]
            mu = jnp.mean(x, axis=0, keepdims=True)
            xc = x - mu
            var = jnp.mean(xc * xc, axis=0, keepdims=True)
            xn = (xc * lax.rsqrt(var + EPS)).astype(BF16)
            kT = _dot(wqkvT_ref[li, D:2 * D, :], xn)
            st_ref[1] = jnp.maximum(st_ref[1], head_norm2(kT))
            kk = kT.T.astype(BF16)
            for g in range(NG):
                k_ref[g, pl.ds(WIN + t0, TT), :] = kk[:, g * T:(g + 1) * T]
            if full:
                for c in range(TT // T):
                    build_kb(kb0_ref, kk[c * T:c * T + VK, 0:T].astype(F32),
                             t * (TT // T) + c, 0, T)
            q = _dot(wqkvT_ref[li, 0:D, :], xn) * QSCALE
            st_ref[0] = jnp.maximum(st_ref[0], head_norm2(q))
            v = _dot(wqkvT_ref[li, 2 * D:3 * D, :], xn)
            st_ref[2] = jnp.maximum(
                st_ref[2], jnp.max(jnp.abs(v).reshape(D // 8, 8, TT), axis=0))
            for c in range(TT // T):
                qT_ref[t * (TT // T) + c] = q[:, c * T:(c + 1) * T].astype(BF16)
                vT_ref[PT + t * (TT // T) + c] = v[:, c * T:(c + 1) * T].astype(BF16)
            return carry
        lax.fori_loop(0, S // TT, body, 0)
        qk2 = jnp.max(st_ref[0]) * jnp.max(st_ref[1])
        vm = jnp.max(st_ref[2])
        return (qk2 * 1.05 <= SMAX * SMAX) & (vm <= VMAX) & (vm >= VMIN)

    def proj_out(li):
        def body(t, carry):
            t0 = pl.multiple_of(t * TT, TT)
            y = _dot(woT_ref[li], oT_ref[:, pl.ds(t0, TT)])
            xT_ref[:, pl.ds(t0, TT)] = xT_ref[:, pl.ds(t0, TT)] + y
            return carry
        lax.fori_loop(0, S // TT, body, 0)

    def q_weights(g, half, qi):
        cols = []
        for j in range(4):
            hh = 4 * half + j
            parts = []
            if hh > 0:
                parts.append(jnp.zeros((8 * hh, T), U32))
            parts.append(qu[qi, pl.ds(_mul(g, T // 2) + 8 * hh, 8), :])
            if hh < 7:
                parts.append(jnp.zeros((8 * (7 - hh), T), U32))
            cols.append(jnp.concatenate(parts, axis=0))
        return _bf(jnp.concatenate(cols, axis=1))

    def _mul(a, n):
        return a * n if isinstance(a, int) else pl.multiple_of(a * n, n)

    def k_rows(g, kt, r0, r1):
        return _bf(ku[g, pl.ds(_mul(kt, T // 2) + r0 // 2, (r1 - r0) // 2), :])

    def v_rows(g, hh, kt):
        return _bf(vu[kt, pl.ds(_mul(g, T // 2) + 8 * hh, 8), :])

    def store_o(g, hh, qi, val):
        oT_ref[pl.ds(_mul(g, T) + DH * hh, DH), pl.ds(_mul(qi, T), T)] = val.astype(BF16)

    def block_max(qk_items, pv_items, nk, slot_of, bias):
        n_items = len(qk_items if qk_items is not None else pv_items)
        lprev = None
        for u in range(n_items):
            sb, srow = slot_of(u)
            if qk_items is not None:
                g1, half1, q1, k1 = qk_items[u]
                w = q_weights(g1, half1, q1)
                m = None
            if pv_items is not None:
                g2, half2, q2, k2 = pv_items[u]
                mprev = m_ref[u]
                acc = [None] * 4
                ls = []

            def expo(c):
                sp = s_ref[sb, srow + c * T:srow + (c + 1) * T, :].reshape(T // 8, 8, 4 * T)
                mp = mprev
                dep = None
                if c >= LAG:
                    dep = ls[c - LAG]
                elif lprev is not None:
                    dep = lprev[c - LAG]
                if dep is not None:
                    mp = jnp.minimum(mprev, jnp.maximum(dep, jnp.inf))
                p = jnp.exp2(sp - mp[None])
                ps = jnp.sum(p, axis=0)
                ls.append(ps if not ls else ls[-1] + ps)
                p = p.reshape(T, 4 * T)
                return [p[:, j * T:(j + 1) * T].astype(BF16) for j in range(4)]

            if pv_items is not None:
                pb = expo(0)
            for c in range(nk):
                if qk_items is not None:
                    s = _dot(k_rows(g1, k1 + c, 0, T), w)
                    if bias is not None:
                        b = bias[c * T:(c + 1) * T, :]
                        s = s + jnp.concatenate([b] * 4, axis=1)
                    s_ref[sb, srow + c * T:srow + (c + 1) * T, :] = s
                    sm = jnp.max(s.reshape(T // 8, 8, 4 * T), axis=0)
                    m = sm if m is None else jnp.maximum(m, sm)
                if pv_items is not None:
                    pb_next = expo(c + 1) if c + 1 < nk else None
                    for j in range(4):
                        o = _dot(v_rows(g2, 4 * half2 + j, k2 + c), pb[j])
                        acc[j] = o if acc[j] is None else acc[j] + o
                    pb = pb_next
            if qk_items is not None:
                m_ref[u] = jnp.broadcast_to(jnp.max(m, axis=0, keepdims=True), (8, 4 * T))
            if pv_items is not None:
                linv = 1.0 / jnp.sum(ls[-1], axis=0, keepdims=True)
                for j in range(4):
                    store_o(g2, 4 * half2 + j, q2, acc[j] * linv[:, j * T:(j + 1) * T])
                lprev = ls

    def block_fast(qk_items, pv_items, nk, slot_of, bias, par):
        n_items = len(qk_items if qk_items is not None else pv_items)
        vk = 0 if par is None else VK
        lastdep = None
        if vk and qk_items is not None:
            g1, _, q1, k1 = qk_items[0]
            qs = _bf(qu[q1, pl.ds(_mul(g1, T // 2), T // 2), :]).astype(F32)
            for d in range(T):
                qb_ref[d] = jnp.broadcast_to(qs[d:d + 1, :], (8, T))
            kb = kbs[par]
            gn = jnp.minimum(g1 + 1, NG - 1)
            kn = k_rows(gn, k1 + q1, 0, VK).astype(F32)
        for u in range(n_items):
            sb, srow = slot_of(u)
            if qk_items is not None:
                g1, half1, q1, k1 = qk_items[u]
                w = q_weights(g1, half1, q1)
                l = [None] * 4
            if pv_items is not None:
                g2, half2, q2, k2 = pv_items[u]
                lprev = m_ref[u]
                acc = [None] * 4

            def vpu_scores(hh, c, dep):
                a = [None] * (VK // 8)
                for d in range(DH):
                    qd = qb_ref[DH * hh + d]
                    if d == 0 and dep is not None:
                        qd = jnp.minimum(qd, dep)
                    for i in range(VK // 8):
                        t = kb[c, DH * hh + d, i * 8:(i + 1) * 8, :] * qd
                        a[i] = t if a[i] is None else a[i] + t
                return jnp.concatenate(a, axis=0)

            for c in range(nk):
                rows = slice(srow + c * T, srow + (c + 1) * T)
                if qk_items is not None:
                    s = _dot(k_rows(g1, k1 + c, vk, T), w)
                if pv_items is not None:
                    for j in range(4):
                        pj = _bf(pu[sb, j, (srow + c * T) // 2:(srow + (c + 1) * T) // 2, :])
                        o = _dot(v_rows(g2, 4 * half2 + j, k2 + c), pj)
                        acc[j] = o if acc[j] is None else acc[j] + o
                if qk_items is not None:
                    if vk:
                        n = u * nk + c
                        nd = T // (n_items * nk)
                        built = build_kb(kbs[1 - par], kn, q1, n * nd, (n + 1) * nd)
                    for j in range(4):
                        sj = s[:, j * T:(j + 1) * T]
                        if bias is not None:
                            sj = sj + bias[c * T:(c + 1) * T, :]
                        if vk:
                            dep = None
                            if lastdep is not None:
                                rr = (j * (lastdep.shape[0] // 8)) // 4
                                dep = jnp.maximum(lastdep[rr * 8:(rr + 1) * 8, 0:T], jnp.inf)
                            sj = jnp.concatenate([vpu_scores(4 * half1 + j, c, dep), sj], axis=0)
                        pj = jnp.exp2(sj)
                        ps = jnp.sum(pj.reshape(T // 8, 8, T), axis=0)
                        l[j] = ps if l[j] is None else l[j] + ps
                        p_ref[sb, j, rows, :] = pj.astype(BF16)
                    lastdep = s
            if qk_items is not None:
                m_ref[u] = jnp.concatenate(
                    [1.0 / jnp.broadcast_to(jnp.sum(l[j], axis=0, keepdims=True), (8, T))
                     for j in range(4)], axis=1)
            if pv_items is not None:
                for j in range(4):
                    li = lprev[:, j * T:(j + 1) * T]
                    store_o(g2, 4 * half2 + j, q2, acc[j] * jnp.concatenate([li, li], axis=0))

    def full_items(g, q):
        return [(g, half, q, PT) for half in range(2)]

    def full_items_b(b):
        if isinstance(b, int):
            return full_items(b // NT, b % NT)
        return full_items(lax.shift_right_logical(b, 4), lax.bitwise_and(b, NT - 1))

    full_slot = lambda u: (u, 0)

    def attn_full_max():
        nb = NG * NT
        block_max(full_items_b(0), None, NT, full_slot, None)

        def body(b, carry):
            block_max(full_items_b(b + 1), full_items_b(b), NT, full_slot, None)
            return carry
        lax.fori_loop(0, nb - 1, body, 0)
        block_max(None, full_items_b(nb - 1), NT, full_slot, None)

    def attn_full_fast():
        block_fast(full_items(0, 0), None, NT, full_slot, None, 0)

        def outer(gp, carry):
            for par in range(2):
                g = 2 * gp + par

                def body(qi, c2, g=g, par=par):
                    block_fast(full_items(g, qi), full_items_b(g * NT + qi - 1),
                               NT, full_slot, None, par)
                    return c2
                lo = jnp.where(gp == 0, 1, 0) if par == 0 else 0
                lax.fori_loop(lo, NT, body, 0)
            return carry
        lax.fori_loop(0, NG // 2, outer, 0)
        block_fast(None, full_items(NG - 1, NT - 1), NT, full_slot, None, 0)

    def attn_window(block):
        def items(b):
            return [(g, half, b, b) for g in range(NG) for half in range(2)]
        slot = lambda u: (u // 4, (u % 4) * 3 * T)
        block(items(0), None, 3, slot, bias_ref.at[0])

        def body(b, carry):
            block(items(b + 1), items(b), 3, slot, bias_ref.at[jnp.minimum(b + 1, 2)])
            return carry
        lax.fori_loop(0, NT - 1, body, 0)
        block(None, items(NT - 1), 3, slot, None)

    def two_layers(_, carry):
        ok = proj_in(0, False)
        pl.when(ok)(lambda: attn_window(
            lambda a, b, c, d, e: block_fast(a, b, c, d, e, None)))
        pl.when(jnp.logical_not(ok))(lambda: attn_window(block_max))
        proj_out(0)
        ok = proj_in(1, True)
        pl.when(ok)(attn_full_fast)
        pl.when(jnp.logical_not(ok))(attn_full_max)
        proj_out(1)
        return carry
    lax.fori_loop(0, 2, two_layers, 0)

    for t in range(S // TT):
        out_ref[t * TT:(t + 1) * TT, :] = xT_ref[:, t * TT:(t + 1) * TT].T.astype(BF16)


@jax.jit
def pallas_interleave_layers__sliding_block__mha_block__prompt_kernel(
    A_x: jax.Array,
    A_wqkv: jax.Array,
    A_wo: jax.Array,
    B_x: jax.Array,
    B_wqkv: jax.Array,
    B_wo: jax.Array,
):
    del B_x
    x = A_x.reshape(S, D)
    out = pl.pallas_call(
        _kernel,
        out_shape=jax.ShapeDtypeStruct((S, D), A_x.dtype),
        scratch_shapes=[
            pltpu.VMEM((D, S), F32),
            pltpu.VMEM((2, 3 * D, D), BF16),
            pltpu.VMEM((2, D, D), BF16),
            pltpu.VMEM((NT, D, T), BF16),
            pltpu.VMEM((NG, S + WIN, T), BF16),
            pltpu.VMEM((NT + PT, D, T), BF16),
            pltpu.VMEM((D, S), BF16),
            pltpu.VMEM((2, S, 4 * T), F32),
            pltpu.VMEM((8, 8, 4 * T), F32),
            pltpu.VMEM((3, 3 * T, T), F32),
            pltpu.VMEM((2, 4, S, T), BF16),
            pltpu.VMEM((T, 8, T), F32),
            pltpu.VMEM((NT, T, VK, T), F32),
            pltpu.VMEM((NT, T, VK, T), F32),
            pltpu.VMEM((3, 8, TT), F32),
        ],
        compiler_params=pltpu.CompilerParams(vmem_limit_bytes=110 * 1024 * 1024),
        name="interleave_attn",
    )(x, A_wqkv, A_wo, B_wqkv, B_wo)
    return out.reshape(A_x.shape)
```

```python
import math

import jax
import jax.numpy as jnp
from jax import lax
import jax.experimental.pallas as pl
import jax.experimental.pallas.tpu as pltpu

S = 2048
D = 512
H = 32
DH = 16
WIN = 256
EPS = 1e-5

T = 128
NT = S // T
NG = D // T
PT = WIN // T
NEG = -1e30
QSCALE = (DH ** -0.5) * math.log2(math.e)
TT = 512
HT = TT // 2
NX = S // TT

SMAX = 60.0
VMAX = 2.0 ** 50
VMIN = 2.0 ** -40

QB = 2
VK = 16
XT = 13
PPC = TT // T + 1
NPIECE = NX * PPC
PIECE = [(c // (TT // T)) * PPC + c % (TT // T) for c in range(NT)]
XPIECE = (XT // (TT // T)) * PPC + TT // T
XPOS = 11
XREL = (4, 6, 8, 10)
DELAY = 9
NCARRY = 2
NS = 4
SQ = T // NS
WCH = (0, 96, 192, 288)
WQ = 4
NWP = 5 * D // T

F32 = jnp.float32
BF16 = jnp.bfloat16
U32 = jnp.uint32


def _dot(a, b):
    return jnp.dot(a, b, preferred_element_type=F32)


def _bf(x):
    return pltpu.bitcast(x, BF16)


def _mul(a, n):
    return a * n if isinstance(a, int) else pl.multiple_of(a * n, n)


def _kernel(x_hbm, awqkv_hbm, awo_hbm, bwqkv_hbm, bwo_hbm, out_hbm,
            x_ref, wa_ref, wb2_ref, sems, xT_ref, waT_ref, wbT_ref,
            qT_ref, k_ref, kh_ref, vT_ref, oT_ref, s_ref, m_ref, bias_ref, wb_ref,
            p_ref, qb_ref, kb0_ref, kb1_ref, kf_ref, cp_ref, ca_ref, st_ref, ok_ref):
    qu = qT_ref.bitcast(U32)
    ku = k_ref.bitcast(U32)
    khu = kh_ref.bitcast(U32)
    vu = vT_ref.bitcast(U32)
    pu = p_ref.bitcast(U32)
    kbs = (kb0_ref, kb1_ref)

    def x_copy(t):
        return pltpu.make_async_copy(x_hbm.at[pl.ds(t * TT, TT)],
                                     x_ref.at[pl.ds(t * TT, TT)], sems.at[t])

    def out_copy(i):
        return pltpu.make_async_copy(x_ref.at[pl.ds(i * HT, HT)],
                                     out_hbm.at[pl.ds(i * HT, HT)], sems.at[i])

    wa_copy = pltpu.make_async_copy(awqkv_hbm, wa_ref, sems.at[NX])
    wb_copies = [
        pltpu.make_async_copy(awo_hbm, wb2_ref.at[:, 0:D], sems.at[NX + 1]),
        pltpu.make_async_copy(bwqkv_hbm, wb2_ref.at[:, D:4 * D], sems.at[NX + 2]),
        pltpu.make_async_copy(bwo_hbm, wb2_ref.at[:, 4 * D:5 * D], sems.at[NX + 3]),
    ]

    def wqkv_t(li, j):
        return waT_ref[j * D:(j + 1) * D, :] if li == 0 else wbT_ref[(j + 1) * D:(j + 2) * D, :]

    def wo_t(li):
        return wbT_ref[0:D, :] if li == 0 else wbT_ref[4 * D:5 * D, :]

    def transpose_wb(piece):
        c0 = _mul(piece, T)
        wbT_ref[pl.ds(c0, T), :] = wb2_ref[:, pl.ds(c0, T)].astype(F32).T.astype(BF16)

    wa_copy.start()
    for t in range(NX):
        x_copy(t).start()
    for g in range(NG):
        k_ref[g, 0:WIN, :] = jnp.zeros((WIN, T), BF16)
    for c in range(PT):
        vT_ref[c] = jnp.zeros((NG, T, T), BF16)
    row = lax.broadcasted_iota(jnp.int32, (3 * T, T), 0)
    col = lax.broadcasted_iota(jnp.int32, (3 * T, T), 1)
    band = (row > col) & (row <= col + WIN)
    for v in range(3):
        bias_ref[v] = jnp.where(band & (row >= WIN - v * T), 0.0, NEG).astype(F32)
    row = lax.broadcasted_iota(jnp.int32, (WIN + SQ, T), 0)
    col = lax.broadcasted_iota(jnp.int32, (WIN + SQ, T), 1) % SQ
    band = (row > col) & (row <= col + WIN)
    for v in range(2 * NS + 1):
        wb_ref[v] = jnp.where(band & (row >= WIN - v * SQ), 0.0, NEG).astype(F32)
    p_ref[NG - 1] = jnp.zeros(p_ref.shape[1:], BF16)
    m_ref[...] = jnp.zeros(m_ref.shape, F32)
    cp_ref[...] = jnp.zeros(cp_ref.shape, F32)
    ca_ref[...] = jnp.zeros(ca_ref.shape, F32)
    oT_ref[...] = jnp.zeros(oT_ref.shape, BF16)

    def head_norm2(a):
        n2 = jnp.sum((a * a).reshape(H, DH, HT), axis=1)
        return jnp.max(n2.reshape(H // 8, 8, HT), axis=0)

    def residual(lo, h0):
        return xT_ref[:, pl.ds(h0, HT)] + _dot(wo_t(lo), oT_ref[:, pl.ds(h0, HT)])

    def normalize(lo, h0):
        if lo is None:
            x = x_ref[pl.ds(h0, HT), :].astype(F32).T
        else:
            x = residual(lo, h0)
        xT_ref[:, pl.ds(h0, HT)] = x
        mu = jnp.mean(x, axis=0, keepdims=True)
        xc = x - mu
        var = jnp.mean(xc * xc, axis=0, keepdims=True)
        return (xc * lax.rsqrt(var + EPS)).astype(BF16)

    def qkv(li, t, hf, xn):
        full = li == 1
        h0 = _mul(t, TT) + hf * HT
        c0 = t * (TT // T) + hf * (HT // T)
        kT = _dot(wqkv_t(li, 1), xn)
        st_ref[1] = jnp.maximum(st_ref[1], head_norm2(kT))
        kf = kT.T
        kk = kf.astype(BF16)
        for g in range(NG):
            k_ref[g, pl.ds(WIN + h0, HT), :] = kk[:, g * T:(g + 1) * T]
        if full:
            for g in range(NG):
                kh_ref[g, pl.ds(h0, HT), :] = pltpu.roll(
                    kf[:, g * T:(g + 1) * T], T // 2, 1).astype(BF16)
            for c in range(HT // T):
                cl = hf * (HT // T) + c
                pieces = [(cl, c * T)]
                if cl == XT % (TT // T):
                    pieces.append((TT // T, c * T + VK))
                for slot, r0 in pieces:
                    piece = t * PPC + slot
                    for g in range(NG):
                        kf_ref[g, piece] = kk[r0:r0 + VK, g * T:(g + 1) * T].astype(F32)
                    kp = kk[r0:r0 + VK, 0:T].astype(F32)
                    for d in range(T):
                        kb0_ref[piece, d] = jnp.broadcast_to(kp[:, d:d + 1], (VK, T))
        q = _dot(wqkv_t(li, 0), xn) * QSCALE
        st_ref[0] = jnp.maximum(st_ref[0], head_norm2(q))
        for c in range(HT // T):
            qc = q[:, c * T:(c + 1) * T]
            if not full:
                qc = jnp.concatenate(
                    [pltpu.roll(qc[DH * h:DH * (h + 1)], SQ * (h % NS), 1)
                     if h % NS else qc[DH * h:DH * (h + 1)] for h in range(H)], axis=0)
            qc = qc.astype(BF16)
            for g in range(NG):
                qT_ref[c0 + c, g] = qc[g * T:(g + 1) * T]
        v = _dot(wqkv_t(li, 2), xn)
        st_ref[2] = jnp.maximum(
            st_ref[2], jnp.max(jnp.abs(v).reshape(D // 8, 8, HT), axis=0))
        for c in range(HT // T):
            for g in range(NG):
                vT_ref[PT + c0 + c, g] = (
                    v[g * T:(g + 1) * T, c * T:(c + 1) * T].astype(BF16))

    def project(lo, li):
        st_ref[...] = jnp.zeros(st_ref.shape, F32)
        if lo is None:
            x_copy(0).wait()

            def body(t, xn0):
                tn = jnp.minimum(t + 1, NX - 1)
                pl.when(t + 1 < NX)(lambda: x_copy(tn).wait())
                xn1 = normalize(None, _mul(t, TT) + HT)
                qkv(li, t, 0, xn0)
                nxt = normalize(None, _mul(tn, TT))
                qkv(li, t, 1, xn1)
                return nxt
            lax.fori_loop(0, NX, body, normalize(None, 0))
        else:
            def body(t, carry):
                xns = [normalize(lo, _mul(t, TT) + hf * HT) for hf in range(2)]
                for hf in range(2):
                    qkv(li, t, hf, xns[hf])
                return carry
            lax.fori_loop(0, NX, body, 0)
        qk2 = jnp.max(st_ref[0]) * jnp.max(st_ref[1])
        vm = jnp.max(st_ref[2])
        ok = (qk2 * 1.05 <= SMAX * SMAX) & (vm <= VMAX) & (vm >= VMIN)
        ok_ref[0] = ok.astype(jnp.int32)

    def finish(lo):
        def body(t, carry):
            for hf in range(4):
                i = 4 * t + hf
                x_ref[pl.ds(_mul(i, HT), HT), :] = residual(lo, _mul(i, HT)).T.astype(BF16)
                out_copy(i).start()
            return carry
        lax.fori_loop(0, S // (4 * HT), body, 0)
        for i in range(S // HT):
            out_copy(i).wait()

    def q_weights(g, heads, qi, rotated=False, base=0):
        cols = []
        for hh in heads:
            parts = []
            if hh > base:
                parts.append(jnp.zeros((8 * (hh - base), T), U32))
            slab = qu[qi, g, 8 * hh:8 * (hh + 1), :]
            if rotated and hh % NS:
                slab = pltpu.roll(slab, T - SQ * (hh % NS), 1)
            parts.append(slab)
            if hh - base < 7:
                parts.append(jnp.zeros((8 * (7 - hh + base), T), U32))
            cols.append(jnp.concatenate(parts, axis=0))
        return _bf(jnp.concatenate(cols, axis=1))

    def v_rows(g, hh, kt):
        return _bf(vu[kt, g, 8 * hh:8 * (hh + 1), :])

    def store_o(g, hh, qi, val):
        oT_ref[pl.ds(_mul(g, T) + DH * hh, DH), pl.ds(_mul(qi, T), T)] = val.astype(BF16)

    def attend_max(g, q, k0, nc, ct, bias):
        ck = ct * T
        for half in range(2):
            heads = range(4 * half, 4 * half + 4)
            w = q_weights(g, heads, q, rotated=bias is not None)

            def scores(i, m):
                sc = _dot(_bf(ku[g, pl.ds(_mul(k0 + i * ct, T // 2), ck // 2), :]), w)
                if bias is not None:
                    sc = sc + jnp.concatenate([bias[...]] * 4, axis=1)
                s_ref[pl.ds(_mul(i, ck), ck), :] = sc
                return jnp.maximum(m, jnp.max(sc.reshape(ck // 8, 8, 4 * T), axis=0))
            m = lax.fori_loop(0, nc, scores, jnp.full((8, 4 * T), -jnp.inf, F32))
            m = jnp.max(m, axis=0, keepdims=True)

            def weigh(i, carry):
                l, acc = carry
                p = jnp.exp2(s_ref[pl.ds(_mul(i, ck), ck), :] - m)
                l = l + jnp.sum(p.reshape(ck // 8, 8, 4 * T), axis=0)
                acc = list(acc)
                for j, hh in enumerate(heads):
                    for c in range(ct):
                        acc[j] = acc[j] + _dot(
                            v_rows(g, hh, k0 + i * ct + c),
                            p[c * T:(c + 1) * T, j * T:(j + 1) * T].astype(BF16))
                return l, tuple(acc)
            l, acc = lax.fori_loop(
                0, nc, weigh,
                (jnp.zeros((8, 4 * T), F32), (jnp.zeros((DH, T), F32),) * 4))
            linv = 1.0 / jnp.sum(l, axis=0, keepdims=True)
            for j, hh in enumerate(heads):
                store_o(g, hh, q, acc[j] * linv[:, j * T:(j + 1) * T])

    def attn_max(window):
        def body(b, carry):
            g = lax.shift_right_logical(b, 4)
            q = lax.bitwise_and(b, NT - 1)
            if window:
                attend_max(g, q, q, 1, 3, bias_ref.at[jnp.minimum(q, 2)])
            else:
                attend_max(g, q, PT, NT // 4, 4, None)
            return carry
        lax.fori_loop(0, NG * NT, body, 0)
        if window:
            def tr(piece, carry):
                transpose_wb(piece)
                return carry
            lax.fori_loop(0, NWP, tr, 0)

    carry_acc = [None] * 4

    def finish_carry(item, i):
        g, half, q = item
        for j in range(4):
            o = _dot(v_rows(g, 4 * half + j, PT + NT - NCARRY + i), cp_ref[i, j])
            carry_acc[j] = (ca_ref[j] if i == 0 else carry_acc[j]) + o
            if i == NCARRY - 1:
                linv = 1.0 / jnp.sum(m_ref[0, :, j * T:(j + 1) * T], axis=0, keepdims=True)
                store_o(g, 4 * half + j, q, carry_acc[j] * linv)

    def build_qb(item, slot, step):
        g, half, q = item
        hh = 4 * half + step // 4
        qs = _bf(qu[q, g, 8 * hh:8 * (hh + 1), :]).astype(F32)
        for r in range(4 * step, 4 * step + 4):
            qb_ref[slot, r] = jnp.broadcast_to(qs[r % DH:r % DH + 1, :], (8, T))

    def block_full(items, prev_item, next_items, blk, par):
        g = items[0][0]
        kb = kbs[par]
        gn = jnp.minimum(g + 1, NG - 1)
        n_items = len(items)
        ngr = T // 16
        order = [c for c in range(NT) if c != XT]
        order.insert(XPOS, XT)
        use = {c: [PIECE[c], XPIECE] if c == XT else [PIECE[c]] for c in range(NT)}
        tiles = [(u, c) for u in range(n_items) for c in order]
        stream = [(u, c, gr) for (u, c) in tiles
                  for gr in range(ngr - 1, len(use[c]) - 1, -1)]
        end = {(u, c): n + 1 for n, (u, c, _) in enumerate(stream)}
        slots = {end[tiles[0]] + DELAY - (NCARRY - i) * (ngr - 1): i for i in range(NCARRY)}
        for t in tiles[:len(tiles) - NCARRY]:
            slots[end[t] + DELAY] = t
        cuts = sorted(set(slots) | {end[(u, NT - 1)] for u in range(n_items)})
        release = [[(u, j, PIECE[c]) for j in range(4)] for (u, c) in tiles]
        for u in range(n_items):
            for j in range(4):
                release[u * NT + XREL[j]].append((u, j, XPIECE))
        spl = len(tiles) * (NT // QB) // T
        ws, sres, l, acc, probs, vres = {}, {}, {}, {}, {}, {}
        lastdep, lastbuilt, lastextra = None, [], []

        def vpu_scores(u, j, piece, dep):
            hh = 4 * items[u][1] + j
            kv = kb[piece, DH * hh:DH * (hh + 1)].reshape(DH, VK // 8, 8, T)
            qv = qb_ref[u, DH * j:DH * (j + 1)]
            if dep is not None:
                qv = jnp.concatenate([jnp.minimum(qv[0:1], dep[None]), qv[1:]], axis=0)
            return jnp.sum(kv * qv[:, None], axis=0).reshape(VK, T)

        def do_pv(u, c):
            _, half, q = items[u]
            ps = probs.pop((u, c))
            for j in range(4):
                o = _dot(v_rows(g, 4 * half + j, PT + c), ps[j])
                acc[(u, j)] = o if c == 0 else acc[(u, j)] + o
                if c == NT - 1:
                    linv = 1.0 / jnp.sum(l[(u, j)], axis=0, keepdims=True)
                    store_o(g, 4 * half + j, q, acc[(u, j)] * linv)

        x = 0
        for y in cuts:
            ch = stream[x:y]
            x = y
            u = ch[0][0]
            _, half, q = items[u]
            if u not in ws:
                ws[u] = q_weights(g, range(4 * half, 4 * half + 4), q, base=4 * half)
            ksrc, koff = (khu, 0) if half else (ku, PT)
            lhs = jnp.concatenate(
                [ksrc[g, (koff + c) * (T // 2) + 8 * gr:(koff + c) * (T // 2) + 8 * gr + 8, :]
                 for (_, c, gr) in ch], axis=0)
            sc = _dot(_bf(lhs), ws[u])
            if y in slots:
                if isinstance(slots[y], int):
                    finish_carry(prev_item, slots[y])
                else:
                    do_pv(*slots[y])
            for n, key in enumerate(ch):
                sres[key] = sc[16 * n:16 * (n + 1)]
            for (_, c, gr) in ch:
                nv = len(use[c])
                if gr != nv:
                    continue
                n = tiles.index((u, c))
                st = jnp.concatenate([sres.pop((u, c, gg)) for gg in range(nv, ngr)], axis=0)
                d = blk * (len(tiles) // spl) + n // spl
                pa = (n % spl) * PPC
                pb = max(pa + PPC - 1, XPIECE + 1) if pa <= XPIECE < pa + PPC else pa + PPC - 1
                src = kf_ref[gn, pa:pb].reshape((pb - pa) * VK, T)
                colv = jnp.take_along_axis(
                    src, jnp.full(src.shape, d, jnp.int32), axis=1, mode="promise_in_bounds")
                for i in range(pb - pa):
                    kbs[1 - par][pa + i, d] = colv[i * VK:(i + 1) * VK]
                built = [colv[8 * i:8 * i + 8] for i in range((pb - pa) * VK // 8)]
                if u < 2:
                    build_qb(items[n_items - 2 + u], n_items - 2 + u, n % NT)
                else:
                    build_qb(next_items[u - 2], u - 2, n % NT)
                todo = release[n]
                for e, unit in enumerate(todo):
                    dep = None
                    if lastdep is not None:
                        nr = lastdep.shape[0] // 8
                        rr = nr - 1 - (e * nr) // len(todo)
                        dep = jnp.maximum(lastdep[rr * 8:(rr + 1) * 8, 0:T], lastbuilt[e])
                        if e == 1:
                            for xr in lastextra:
                                dep = jnp.maximum(dep, jnp.maximum(xr[0:8], xr[8:16]))
                        dep = jnp.maximum(dep, jnp.inf)
                    vres[unit] = vpu_scores(*unit, dep)
                lastextra = [vres[unit] for unit in todo[4:]]
                ps = []
                for j in range(4):
                    parts = [vres.pop((u, j, piece)) for piece in use[c]]
                    pj = jnp.exp2(jnp.concatenate(parts + [st[:, j * T:(j + 1) * T]], axis=0))
                    cur = None if c == 0 else l[(u, j)]
                    for gg in range(ngr - 1, -1, -1):
                        for hf in range(2):
                            pr = pj[16 * gg + 8 * hf:16 * gg + 8 * hf + 8]
                            cur = pr if cur is None else cur + pr
                    l[(u, j)] = cur
                    ps.append(pj)
                if n >= len(tiles) - NCARRY:
                    for j in range(4):
                        cp_ref[n - (len(tiles) - NCARRY), j] = ps[j]
                else:
                    probs[(u, c)] = ps
                lastdep, lastbuilt = st, built
        for j in range(4):
            ca_ref[j] = acc[(n_items - 1, j)]
            m_ref[0, :, j * T:(j + 1) * T] = l[(n_items - 1, j)]

    def attn_full_fast():
        nb = NT // QB

        def items(g, blk):
            return [(g, half, blk * QB + dq) for dq in range(QB) for half in range(2)]

        def items_at(b):
            return items(lax.shift_right_logical(b, nb.bit_length() - 1),
                         lax.bitwise_and(b, nb - 1))

        for u, item in enumerate(items(0, 0)[:-2]):
            for step in range(NT):
                build_qb(item, u, step)

        def outer(gp, carry):
            for par in range(2):
                g = 2 * gp + par

                def body(blk, c2, g=g, par=par):
                    prev = items_at(jnp.maximum(g * nb + blk - 1, 0))[-1]
                    nxt = items_at(jnp.minimum(g * nb + blk + 1, NG * nb - 1))
                    block_full(items(g, blk), prev, nxt, blk, par)
                    return c2
                lax.fori_loop(0, nb, body, 0)
            return carry
        lax.fori_loop(0, NG // 2, outer, 0)
        for i in range(NCARRY):
            finish_carry(items(NG - 1, nb - 1)[-1], i)

    def attn_window_fast():
        lane_grp = lax.broadcasted_iota(jnp.int32, (8, T), 1) // SQ
        nset = 8 // NS

        def pick(parts, a0, rows):
            grp = jnp.concatenate([lane_grp] * (rows // 8), axis=0)
            out = parts[0]
            for u in range(1, NS):
                out = jnp.where(grp == (a0 + u) % NS, parts[u], out)
            return out

        def qk_ops(g, b):
            slabs = [qu[b, g, 8 * hh:8 * (hh + 1), :] for hh in range(8)]
            zero = jnp.zeros((8, T), U32)
            state = {}

            def run(u, i):
                if i == 0:
                    tiles = [jnp.concatenate(
                        [jnp.where(lane_grp == (hh % NS + u) % NS, slabs[hh], zero)
                         if hh // NS == sg else zero for hh in range(8)], axis=0)
                        for sg in range(nset)]
                    state[u] = (_bf(jnp.concatenate(tiles, axis=1)), [None] * nset)
                w, l = state[u]
                r0, r1 = WCH[i], WCH[i + 1]
                kwin = ku.at[g, pl.ds(_mul(b, T // 2), 3 * T // 2)]
                sc = _dot(_bf(kwin[(SQ * u + r0) // 2:(SQ * u + r1) // 2, :]), w)

                def post():
                    bias = wb_ref[jnp.minimum(NS * b + u, 2 * NS), r0:r1, :]
                    for sg in range(nset):
                        p = jnp.exp2(sc[:, sg * T:(sg + 1) * T] + bias)
                        ps = jnp.sum(p.reshape((r1 - r0) // 8, 8, T), axis=0)
                        l[sg] = ps if l[sg] is None else l[sg] + ps
                        p_ref[g, sg * NS + u, r0:r1, :] = p.astype(BF16)
                        if i == len(WCH) - 2:
                            m_ref[nset * g + sg, :, u * T:(u + 1) * T] = l[sg]
                return post

            return [lambda u0=u0, i=i: [run(u, i) for u in (u0, u0 + 1)]
                    for u0 in range(0, NS, 2) for i in range(len(WCH) - 1)]

        def pv_ops(g, b):
            acc = [None] * 8

            def run(hh, c):
                sg, a0 = divmod(hh, NS)
                parts = []
                for u in range(NS):
                    lo = c * T - SQ * u
                    r0, r1 = max(lo, 0), min(lo + T, WIN + SQ)
                    pieces = []
                    if r0 > lo:
                        pieces.append(jnp.zeros(((r0 - lo) // 2, T), U32))
                    pieces.append(pu[g, sg * NS + u, r0 // 2:r1 // 2, :])
                    if lo + T > r1:
                        pieces.append(jnp.zeros(((lo + T - r1) // 2, T), U32))
                    parts.append(jnp.concatenate(pieces, axis=0))
                o = _dot(v_rows(g, hh, b + c), _bf(pick(parts, a0, T // 2)))
                acc[hh] = o if acc[hh] is None else acc[hh] + o
                if c == 2:
                    ls = [m_ref[nset * g + sg, :, u * T:(u + 1) * T] for u in range(NS)]
                    linv = 1.0 / jnp.sum(pick(ls, a0, 8), axis=0, keepdims=True)
                    o = acc[hh] * linv
                    if a0:
                        o = pltpu.roll(o, T - SQ * a0, 1)
                    store_o(g, hh, b, o)

            return [lambda c=c, h0=h0: [run(hh, c) for hh in range(h0, h0 + 4)]
                    for c in range(3) for h0 in (0, 4)]

        def body(bb, carry):
            npc = NWP // (NT // WQ)
            for i in range(npc):
                transpose_wb(bb * npc + i)
            for dq in range(WQ):
                b = bb * WQ + dq
                for g in range(NG):
                    qk = qk_ops(g, b)
                    bp = b if g else (b - 1 if dq else jnp.maximum(b - 1, 0))
                    pv = pv_ops((g - 1) % NG, bp)
                    if dq == WQ - 1 and g == NG - 1:
                        pv = [lambda i=i, pv=pv: [f() for f in pv[2 * i:2 * i + 2]]
                              for i in range(len(pv))]
                    for qk_p, pv_p in zip(qk, pv):
                        posts = qk_p()
                        pv_p()
                        for post in posts:
                            post()
            return carry
        lax.fori_loop(0, NT // WQ, body, 0)
        for pv_p in pv_ops(NG - 1, NT - 1):
            pv_p()

    wa_copy.wait()
    for cp in wb_copies:
        cp.start()
    for j in range(3):
        waT_ref[j * D:(j + 1) * D, :] = (
            wa_ref[:, j * D:(j + 1) * D].astype(F32).T.astype(BF16))
    project(None, 0)
    for cp in wb_copies:
        cp.wait()

    def two_layers(it, carry):
        lax.cond(ok_ref[0] != 0, attn_window_fast, lambda: attn_max(True))
        project(0, 1)
        lax.cond(ok_ref[0] != 0, attn_full_fast, lambda: attn_max(False))
        pl.when(it == 0)(lambda: project(1, 0))
        return carry
    lax.fori_loop(0, 2, two_layers, 0)
    finish(1)


@jax.jit
def pallas_interleave_layers__sliding_block__mha_block__prompt_kernel(
    A_x: jax.Array,
    A_wqkv: jax.Array,
    A_wo: jax.Array,
    B_x: jax.Array,
    B_wqkv: jax.Array,
    B_wo: jax.Array,
):
    del B_x
    x = A_x.reshape(S, D)
    out = pl.pallas_call(
        _kernel,
        out_shape=jax.ShapeDtypeStruct((S, D), A_x.dtype),
        in_specs=[pl.BlockSpec(memory_space=pl.ANY)] * 5,
        out_specs=pl.BlockSpec(memory_space=pl.ANY),
        scratch_shapes=[
            pltpu.VMEM((S, D), BF16),
            pltpu.VMEM((D, 3 * D), BF16),
            pltpu.VMEM((D, 5 * D), BF16),
            pltpu.SemaphoreType.DMA((S // HT,)),
            pltpu.VMEM((D, S), F32),
            pltpu.VMEM((3 * D, D), BF16),
            pltpu.VMEM((5 * D, D), BF16),
            pltpu.VMEM((NT, NG, T, T), BF16),
            pltpu.VMEM((NG, S + WIN, T), BF16),
            pltpu.VMEM((NG, S, T), BF16),
            pltpu.VMEM((NT + PT, NG, T, T), BF16),
            pltpu.VMEM((D, S), BF16),
            pltpu.VMEM((S, 4 * T), F32),
            pltpu.VMEM((8, 8, 4 * T), F32),
            pltpu.VMEM((3, 3 * T, T), F32),
            pltpu.VMEM((2 * NS + 1, WIN + SQ, T), F32),
            pltpu.VMEM((NG, 8, 3 * T, T), BF16),
            pltpu.VMEM((2 * QB, 4 * DH, 8, T), F32),
            pltpu.VMEM((NPIECE, T, VK, T), F32),
            pltpu.VMEM((NPIECE, T, VK, T), F32),
            pltpu.VMEM((NG, NPIECE, VK, T), F32),
            pltpu.VMEM((NCARRY, 4, T, T), F32),
            pltpu.VMEM((4, DH, T), F32),
            pltpu.VMEM((4, 8, HT), F32),
            pltpu.SMEM((1,), jnp.int32),
        ],
        compiler_params=pltpu.CompilerParams(vmem_limit_bytes=100 * 1024 * 1024),
        name="interleave_attn",
    )(x, A_wqkv, A_wo, B_wqkv, B_wo)
    return out.reshape(A_x.shape)
```

```python
import math

import jax
import jax.numpy as jnp
from jax import lax
import jax.experimental.pallas as pl
import jax.experimental.pallas.tpu as pltpu

S = 2048
D = 512
H = 32
DH = 16
WIN = 256
EPS = 1e-5

T = 128
NT = S // T
NG = D // T
PT = WIN // T
NEG = -1e30
QSCALE = (DH ** -0.5) * math.log2(math.e)
TT = 512
HT = TT // 2
NX = S // TT

SMAX = 60.0
VMAX = 2.0 ** 50
VMIN = 2.0 ** -40

QB = 2
VK = 16
PPC = TT // T + 1
NPIECE = NX * PPC
XSLOT = 1
EXTRA = ((13, 12, (5, 7, 9, 11)), (9, 11, (4, 6, 8, 10)))
DELAY = 9
NCARRY = 2
NS = 4
SQ = T // NS
WCH = (0, 96, 192, 288)
WQ = 4
NWP = 5 * D // T

F32 = jnp.float32
BF16 = jnp.bfloat16
U32 = jnp.uint32


def _dot(a, b):
    return jnp.dot(a, b, preferred_element_type=F32)


def _bf(x):
    return pltpu.bitcast(x, BF16)


def _pk(x):
    return pltpu.bitcast(x.astype(BF16), U32)


def _recip(x):
    r = pl.reciprocal(x, approx=True)
    return r * (2.0 - x * r)


def _mul(a, n):
    return a * n if isinstance(a, int) else pl.multiple_of(a * n, n)


def _kernel(x_hbm, awqkv_hbm, awo_hbm, bwqkv_hbm, bwo_hbm, out_hbm,
            x_ref, wa_ref, wb2_ref, sems, xT_ref, waT_ref, wbT_ref,
            qu, ku, khu, vu, oT_ref, s_ref, m_ref, bias_ref, wb_ref,
            p_ref, qb_ref, kb0_ref, kb1_ref, kf_ref, cp_ref, ca_ref, st_ref, ok_ref):
    kbs = (kb0_ref, kb1_ref)

    def x_copy(i):
        return pltpu.make_async_copy(x_hbm.at[pl.ds(i * HT, HT)],
                                     x_ref.at[pl.ds(i * HT, HT)], sems.at[i])

    def out_copy(i):
        return pltpu.make_async_copy(x_ref.at[pl.ds(i * HT, HT)],
                                     out_hbm.at[pl.ds(i * HT, HT)], sems.at[i])

    wa_copies = [pltpu.make_async_copy(awqkv_hbm.at[:, j * D:(j + 1) * D], wa_ref.at[j],
                                       sems.at[2 * NX + 3 + j]) for j in range(3)]
    wb_copies = [
        pltpu.make_async_copy(awo_hbm, wb2_ref.at[:, 0:D], sems.at[2 * NX]),
        pltpu.make_async_copy(bwqkv_hbm, wb2_ref.at[:, D:4 * D], sems.at[2 * NX + 1]),
        pltpu.make_async_copy(bwo_hbm, wb2_ref.at[:, 4 * D:5 * D], sems.at[2 * NX + 2]),
    ]

    def wqkv_t(li, j):
        return waT_ref[j * D:(j + 1) * D, :] if li == 0 else wbT_ref[(j + 1) * D:(j + 2) * D, :]

    def wo_t(li):
        return wbT_ref[0:D, :] if li == 0 else wbT_ref[4 * D:5 * D, :]

    def transpose_wb(piece):
        c0 = _mul(piece, T)
        wbT_ref[pl.ds(c0, T), :] = wb2_ref[:, pl.ds(c0, T)].astype(F32).T.astype(BF16)

    x_copy(0).start()
    for cp in wa_copies:
        cp.start()
    x_copy(1).start()
    x_copy(2).start()
    for g in range(NG):
        ku[g, 0:WIN // 2, :] = jnp.zeros((WIN // 2, T), U32)
    for c in range(PT):
        vu[c] = jnp.zeros((NG, T // 2, T), U32)
    row = lax.broadcasted_iota(jnp.int32, (3 * T, T), 0)
    col = lax.broadcasted_iota(jnp.int32, (3 * T, T), 1)
    band = (row > col) & (row <= col + WIN)
    for v in range(3):
        bias_ref[v] = jnp.where(band & (row >= WIN - v * T), 0.0, NEG).astype(F32)
    row = lax.broadcasted_iota(jnp.int32, (WIN + SQ, T), 0)
    col = lax.broadcasted_iota(jnp.int32, (WIN + SQ, T), 1) % SQ
    band = (row > col) & (row <= col + WIN)
    for v in range(2 * NS + 1):
        wb_ref[v] = jnp.where(band & (row >= WIN - v * SQ), 0.0, NEG).astype(F32)
    p_ref[NG - 1] = jnp.zeros(p_ref.shape[1:], BF16)
    m_ref[...] = jnp.zeros(m_ref.shape, F32)
    cp_ref[...] = jnp.zeros(cp_ref.shape, F32)
    ca_ref[...] = jnp.zeros(ca_ref.shape, F32)
    oT_ref[...] = jnp.zeros(oT_ref.shape, BF16)

    def head_norm2(a):
        n2 = jnp.sum((a * a).reshape(H, DH, HT), axis=1)
        return jnp.max(n2.reshape(H // 8, 8, HT), axis=0)

    def residual(lo, h0):
        return xT_ref[:, pl.ds(h0, HT)] + _dot(wo_t(lo), oT_ref[:, pl.ds(h0, HT)])

    def normalize(lo, h0):
        if lo is None:
            x = x_ref[pl.ds(h0, HT), :].astype(F32).T
        else:
            x = residual(lo, h0)
        xT_ref[:, pl.ds(h0, HT)] = x
        mu = jnp.mean(x, axis=0, keepdims=True)
        xc = x - mu
        var = jnp.mean(xc * xc, axis=0, keepdims=True)
        return (xc * lax.rsqrt(var + EPS)).astype(BF16)

    def qkv(li, t, hf, xn, which):
        for w in which:
            qkv1(li, t, hf, xn, w)

    def qkv1(li, t, hf, xn, which):
        full = li == 1
        hh0 = _mul(t, TT // 2) + hf * (HT // 2)
        c0 = t * (TT // T) + hf * (HT // T)
        if which == 'k':
            kT = _dot(wqkv_t(li, 1), xn)
            st_ref[1] = jnp.maximum(st_ref[1], head_norm2(kT))
            kf = kT.T
            kk = kf.astype(BF16)
            for g in range(NG):
                ku[g, pl.ds(WIN // 2 + hh0, HT // 2), :] = _pk(kf[:, g * T:(g + 1) * T])
            if full:
                for g in range(NG):
                    khu[g, pl.ds(hh0, HT // 2), :] = _pk(
                        pltpu.roll(kf[:, g * T:(g + 1) * T], T // 2, 1))
                for c in range(HT // T):
                    cl = hf * (HT // T) + c
                    pieces = [(cl, c * T)]
                    if cl == XSLOT:
                        pieces.append((TT // T, c * T + VK))
                    for slot, r0 in pieces:
                        piece = t * PPC + slot
                        for g in range(NG):
                            kf_ref[g, piece] = kk[r0:r0 + VK, g * T:(g + 1) * T].astype(F32)
                        kp = kk[r0:r0 + VK, 0:T].astype(F32)
                        kb0_ref[piece] = jnp.stack(
                            [jnp.broadcast_to(kp[:, d:d + 1], (VK, T)) for d in range(T)])
        if which == 'q':
            q = _dot(wqkv_t(li, 0), xn) * QSCALE
            st_ref[0] = jnp.maximum(st_ref[0], head_norm2(q))
            for c in range(HT // T):
                qc = q[:, c * T:(c + 1) * T]
                if not full:
                    qc = jnp.concatenate(
                        [pltpu.roll(qc[DH * h:DH * (h + 1)], SQ * (h % NS), 1)
                         if h % NS else qc[DH * h:DH * (h + 1)] for h in range(H)], axis=0)
                for g in range(NG):
                    qu[c0 + c, g] = _pk(qc[g * T:(g + 1) * T])
        if which == 'v':
            v = _dot(wqkv_t(li, 2), xn)
            st_ref[2] = jnp.maximum(
                st_ref[2], jnp.max(jnp.abs(v).reshape(D // 8, 8, HT), axis=0))
            for c in range(HT // T):
                for g in range(NG):
                    vu[PT + c0 + c, g] = _pk(v[g * T:(g + 1) * T, c * T:(c + 1) * T])

    def project(lo, li):
        st_ref[...] = jnp.zeros(st_ref.shape, F32)
        if lo is None:
            x_copy(0).wait()
            first = normalize(None, 0)
            for j in range(3):
                wa_copies[j].wait()
                waT_ref[j * D:(j + 1) * D, :] = wa_ref[j].astype(F32).T.astype(BF16)

            def body(t, xn0):
                tn = jnp.minimum(t + 1, NX - 1)
                x_copy(2 * t + 1).wait()
                pl.when(t + 1 < NX)(lambda: x_copy(2 * tn).wait())

                @pl.when(t == 0)
                def _():
                    for i in range(3, 2 * NX):
                        x_copy(i).start()
                    for cp in wb_copies:
                        cp.start()
                xn1 = normalize(None, _mul(t, TT) + HT)
                qkv(li, t, 0, xn0, 'qkv')
                nxt = normalize(None, _mul(tn, TT))
                qkv(li, t, 1, xn1, 'qkv')
                return nxt
            lax.fori_loop(0, NX, body, first)
        else:
            def body(t, carry):
                xns = [normalize(lo, _mul(t, TT) + hf * HT) for hf in range(2)]
                for hf in range(2):
                    qkv(li, t, hf, xns[hf], 'kqv')
                return carry
            lax.fori_loop(0, NX, body, 0)
        qk2 = jnp.max(st_ref[0]) * jnp.max(st_ref[1])
        vm = jnp.max(st_ref[2])
        ok = (qk2 * 1.05 <= SMAX * SMAX) & (vm <= VMAX) & (vm >= VMIN)
        ok_ref[0] = ok.astype(jnp.int32)

    def finish(lo):
        def body(t, carry):
            for hf in range(4):
                i = 4 * t + hf
                x_ref[pl.ds(_mul(i, HT), HT), :] = residual(lo, _mul(i, HT)).T.astype(BF16)
                out_copy(i).start()
            return carry
        lax.fori_loop(0, S // (4 * HT), body, 0)
        for i in range(S // HT):
            out_copy(i).wait()

    def q_weights(g, heads, qi, rotated=False, base=0):
        cols = []
        for hh in heads:
            parts = []
            if hh > base:
                parts.append(jnp.zeros((8 * (hh - base), T), U32))
            slab = qu[qi, g, 8 * hh:8 * (hh + 1), :]
            if rotated and hh % NS:
                slab = pltpu.roll(slab, T - SQ * (hh % NS), 1)
            parts.append(slab)
            if hh - base < 7:
                parts.append(jnp.zeros((8 * (7 - hh + base), T), U32))
            cols.append(jnp.concatenate(parts, axis=0))
        return _bf(jnp.concatenate(cols, axis=1))

    def v_rows(g, hh, kt):
        return _bf(vu[kt, g, 8 * hh:8 * (hh + 1), :])

    def v_rows4(g, half, kt):
        vv = vu[kt, g, 32 * half:32 * (half + 1), :]
        return [_bf(vv[8 * j:8 * (j + 1)]) for j in range(4)]

    def store_o(g, hh, qi, val):
        oT_ref[pl.ds(_mul(g, T) + DH * hh, DH), pl.ds(_mul(qi, T), T)] = val.astype(BF16)

    def attend_max(g, q, k0, nc, ct, bias):
        ck = ct * T
        for half in range(2):
            heads = range(4 * half, 4 * half + 4)
            w = q_weights(g, heads, q, rotated=bias is not None)

            def scores(i, m):
                sc = _dot(_bf(ku[g, pl.ds(_mul(k0 + i * ct, T // 2), ck // 2), :]), w)
                if bias is not None:
                    sc = sc + jnp.concatenate([bias[...]] * 4, axis=1)
                s_ref[pl.ds(_mul(i, ck), ck), :] = sc
                return jnp.maximum(m, jnp.max(sc.reshape(ck // 8, 8, 4 * T), axis=0))
            m = lax.fori_loop(0, nc, scores, jnp.full((8, 4 * T), -jnp.inf, F32))
            m = jnp.max(m, axis=0, keepdims=True)

            def weigh(i, carry):
                l, acc = carry
                p = jnp.exp2(s_ref[pl.ds(_mul(i, ck), ck), :] - m)
                l = l + jnp.sum(p.reshape(ck // 8, 8, 4 * T), axis=0)
                acc = list(acc)
                for j, hh in enumerate(heads):
                    for c in range(ct):
                        acc[j] = acc[j] + _dot(
                            v_rows(g, hh, k0 + i * ct + c),
                            p[c * T:(c + 1) * T, j * T:(j + 1) * T].astype(BF16))
                return l, tuple(acc)
            l, acc = lax.fori_loop(
                0, nc, weigh,
                (jnp.zeros((8, 4 * T), F32), (jnp.zeros((DH, T), F32),) * 4))
            linv = 1.0 / jnp.sum(l, axis=0, keepdims=True)
            for j, hh in enumerate(heads):
                store_o(g, hh, q, acc[j] * linv[:, j * T:(j + 1) * T])

    def attn_max(window):
        def body(b, carry):
            g = lax.shift_right_logical(b, 4)
            q = lax.bitwise_and(b, NT - 1)
            if window:
                attend_max(g, q, q, 1, 3, bias_ref.at[jnp.minimum(q, 2)])
            else:
                attend_max(g, q, PT, NT // 4, 4, None)
            return carry
        lax.fori_loop(0, NG * NT, body, 0)
        if window:
            def tr(piece, carry):
                transpose_wb(piece)
                return carry
            lax.fori_loop(0, NWP, tr, 0)

    carry_acc = [None] * 4

    def finalize(item, acc, l):
        g, half, q = item
        linv = _recip(jnp.sum(l, axis=0, keepdims=True))
        o = jnp.concatenate([acc[j] * linv[:, j * T:(j + 1) * T] for j in range(4)], axis=0)
        oT_ref[pl.ds(_mul(g, T) + 4 * DH * half, 4 * DH), pl.ds(_mul(q, T), T)] = o.astype(BF16)

    def finish_carry(item, i):
        vs = v_rows4(item[0], item[1], PT + NT - NCARRY + i)
        for j in range(4):
            o = _dot(vs[j], cp_ref[i, :, j * T:(j + 1) * T])
            carry_acc[j] = (ca_ref[j] if i == 0 else carry_acc[j]) + o
        if i == NCARRY - 1:
            finalize(item, carry_acc, m_ref[0])

    def build_qb(item, slot, step):
        g, half, q = item
        hh = 4 * half + step // 4
        qs = _bf(qu[q, g, 8 * hh:8 * (hh + 1), :]).astype(F32)
        qb_ref[slot, 4 * step:4 * step + 4] = jnp.stack(
            [jnp.broadcast_to(qs[r % DH:r % DH + 1, :], (8, T))
             for r in range(4 * step, 4 * step + 4)])

    def block_full(items, prev_item, next_items, blk, par):
        g = items[0][0]
        kb = kbs[par]
        gn = jnp.minimum(g + 1, NG - 1)
        n_items = len(items)
        ngr = T // 16
        piece = lambda c: (c // (TT // T)) * PPC + c % (TT // T)
        spare = lambda c: (c // (TT // T)) * PPC + TT // T
        order = [None] * NT
        for xt, pos, _ in EXTRA:
            order[pos] = xt
        use = {c: [piece(c), spare(c)] if c in order else [piece(c)] for c in range(NT)}
        rest = [c for c in range(NT) if c not in order]
        order = [c if c is not None else rest.pop(0) for c in order]
        tiles = [(u, c) for u in range(n_items) for c in order]
        stream = [(u, c, gr) for (u, c) in tiles
                  for gr in range(ngr - 1, len(use[c]) - 1, -1)]
        end = {(u, c): n + 1 for n, (u, c, _) in enumerate(stream)}
        slots = {end[tiles[0]] + DELAY - (NCARRY - i) * (ngr - 1): i for i in range(NCARRY)}
        for t in tiles[:len(tiles) - NCARRY]:
            slots[end[t] + DELAY] = t
        cuts = sorted(set(slots) | {end[(u, NT - 1)] for u in range(n_items)})
        release = [[(u, j, piece(c)) for j in range(4)] for (u, c) in tiles]
        for u in range(n_items):
            for xt, _, rel in EXTRA:
                for j in range(4):
                    release[u * NT + rel[j]].append((u, j, spare(xt)))
        spl = len(tiles) * (NT // QB) // T
        ws, sres, l, acc, probs, vres = {}, {}, {}, {}, {}, {}
        always = jnp.full((8, T), ok_ref[0], jnp.int32) != 0
        lastdep, lastbuilt, lastextra = None, [], []

        def vpu_scores(u, j, pc, dep):
            hh = 4 * items[u][1] + j
            kv = kb[pc, DH * hh:DH * (hh + 1)].reshape(DH, VK // 8, 8, T)
            qv = qb_ref[u, DH * j:DH * (j + 1)]
            if dep is not None:
                qv = jnp.concatenate(
                    [jnp.where(always[None], qv[0:1], dep[None]), qv[1:]], axis=0)
            return jnp.sum(kv * qv[:, None], axis=0).reshape(VK, T)

        def do_pv(u, c):
            p = probs.pop((u, c))
            vs = v_rows4(g, items[u][1], PT + c)
            for j in range(4):
                o = _dot(vs[j], p[:, j * T:(j + 1) * T])
                acc[(u, j)] = o if c == 0 else acc[(u, j)] + o
            if c == NT - 1:
                finalize(items[u], [acc[(u, j)] for j in range(4)], l[u])

        x = 0
        for y in cuts:
            ch = stream[x:y]
            x = y
            u = ch[0][0]
            _, half, q = items[u]
            if u not in ws:
                ws[u] = q_weights(g, range(4 * half, 4 * half + 4), q, base=4 * half)
            ksrc, koff = (khu, 0) if half else (ku, PT)
            rows = []
            for c in dict.fromkeys(c for (_, c, _) in ch):
                grs = [gr for (_, cc, gr) in ch if cc == c]
                r0 = (koff + c) * (T // 2) + 8 * grs[-1]
                kt = ksrc[g, r0:r0 + 8 * len(grs), :]
                rows += [kt[8 * (gr - grs[-1]):8 * (gr - grs[-1] + 1)] for gr in grs]
            lhs = jnp.concatenate(rows, axis=0)
            sc = _dot(_bf(lhs), ws[u])
            if y in slots:
                if isinstance(slots[y], int):
                    finish_carry(prev_item, slots[y])
                else:
                    do_pv(*slots[y])
            n0 = 0
            for c in dict.fromkeys(c for (_, c, _) in ch):
                cnt = sum(cc == c for (_, cc, _) in ch)
                sres.setdefault((u, c), []).append(sc[16 * n0:16 * (n0 + cnt)])
                n0 += cnt
            for (_, c, gr) in ch:
                nv = len(use[c])
                if gr != nv:
                    continue
                n = tiles.index((u, c))
                st = jnp.concatenate(sres.pop((u, c)), axis=0)
                d = blk * (len(tiles) // spl) + n // spl
                pa = (n % spl) * PPC
                pb = pa + PPC - (pa + PPC - 1 not in [spare(xt) for xt, _, _ in EXTRA])
                src = kf_ref[gn, pa:pb].reshape((pb - pa) * VK, T)
                colv = jnp.take_along_axis(
                    src, jnp.full(src.shape, d, jnp.int32), axis=1, mode="promise_in_bounds")
                kbs[1 - par][pa:pb, d] = colv.reshape(pb - pa, VK, T)
                built = colv
                if u < 2:
                    build_qb(items[n_items - 2 + u], n_items - 2 + u, n % NT)
                else:
                    build_qb(next_items[u - 2], u - 2, n % NT)
                todo = release[n]
                for e, unit in enumerate(todo):
                    dep = None
                    if lastdep is not None:
                        nr = lastdep.shape[0] // 8
                        rr = ((e * nr) // len(todo)) ^ 1
                        dep = jnp.maximum(lastdep[rr * 8:(rr + 1) * 8, 0:T],
                                          lastbuilt[e * 8:(e + 1) * 8])
                        if e == 0:
                            for xr in lastextra:
                                dep = jnp.maximum(dep, jnp.maximum(xr[0:8], xr[8:16]))
                    vres[unit] = vpu_scores(*unit, dep)
                lastextra = [vres[unit] for unit in todo[4:]]
                parts = [jnp.concatenate([vres.pop((u, j, pc)) for j in range(4)], axis=1)
                         for pc in reversed(use[c])]
                p = jnp.exp2(jnp.concatenate([st] + parts, axis=0))
                if c == 0:
                    l[u] = jnp.sum(p.reshape(T // 8, 8, 4 * T), axis=0)
                else:
                    l[u] = jnp.sum(jnp.concatenate([l[u], p], axis=0).reshape(
                        T // 8 + 1, 8, 4 * T), axis=0)
                p = jnp.concatenate(
                    [p[16 * gg:16 * (gg + 1)] for gg in range(ngr - 1, -1, -1)], axis=0)
                if n >= len(tiles) - NCARRY:
                    cp_ref[n - (len(tiles) - NCARRY)] = p
                else:
                    probs[(u, c)] = p
                lastdep, lastbuilt = st, built
        ca_ref[...] = jnp.stack([acc[(n_items - 1, j)] for j in range(4)])
        m_ref[0] = l[n_items - 1]

    def attn_full_fast():
        nb = NT // QB

        def items(g, blk):
            return [(g, half, blk * QB + dq) for dq in range(QB) for half in range(2)]

        def items_at(b):
            return items(lax.shift_right_logical(b, nb.bit_length() - 1),
                         lax.bitwise_and(b, nb - 1))

        for u, item in enumerate(items(0, 0)[:-2]):
            for step in range(NT):
                build_qb(item, u, step)

        def outer(gp, carry):
            for par in range(2):
                g = 2 * gp + par

                def body(blk, c2, g=g, par=par):
                    prev = items_at(jnp.maximum(g * nb + blk - 1, 0))[-1]
                    nxt = items_at(jnp.minimum(g * nb + blk + 1, NG * nb - 1))
                    block_full(items(g, blk), prev, nxt, blk, par)
                    return c2
                lax.fori_loop(0, nb, body, 0)
            return carry
        lax.fori_loop(0, NG // 2, outer, 0)
        for i in range(NCARRY):
            finish_carry(items(NG - 1, nb - 1)[-1], i)

    def attn_window_fast():
        nset = 8 // NS

        is_grp = {(rows, a): lax.broadcasted_iota(jnp.int32, (rows, T), 1) // SQ == a
                  for rows in (8, T // 2) for a in range(NS)}

        def pick(parts, a0):
            out = parts[0]
            for u in range(1, NS):
                out = jnp.where(is_grp[(out.shape[0], (a0 + u) % NS)], parts[u], out)
            return out

        def qk_ops(g, b, interior):
            qg = qu[b, g]
            slabs = [qg[8 * hh:8 * (hh + 1)] for hh in range(8)]
            zero = jnp.zeros((8, T), U32)
            state = {}

            def run(u, i):
                if i == 0:
                    tiles = [jnp.concatenate(
                        [jnp.where(is_grp[(8, (hh % NS + u) % NS)], slabs[hh], zero)
                         if hh // NS == sg else zero for hh in range(8)], axis=0)
                        for sg in range(nset)]
                    state[u] = (_bf(jnp.concatenate(tiles, axis=1)), [None] * nset)
                w, l = state[u]
                r0, r1 = WCH[i], WCH[i + 1]
                kwin = ku.at[g, pl.ds(_mul(b, T // 2), 3 * T // 2)]
                sc = _dot(_bf(kwin[(SQ * u + r0) // 2:(SQ * u + r1) // 2, :]), w)

                def post():
                    m0 = max(r0, WIN) if interior and r0 >= SQ else r0
                    m1 = min(r1, SQ) if interior and r1 <= WIN else r1
                    if m1 > m0:
                        bias = wb_ref[jnp.minimum(NS * b + u, 2 * NS), m0:m1, :]
                    for sg in range(nset):
                        z = sc[:, sg * T:(sg + 1) * T]
                        if m1 > m0:
                            z = jnp.concatenate(
                                [e for e in (z[:m0 - r0], z[m0 - r0:m1 - r0] + bias, z[m1 - r0:])
                                 if e.shape[0]], axis=0)
                        p = jnp.exp2(z)
                        ps = jnp.sum(p.reshape((r1 - r0) // 8, 8, T), axis=0)
                        l[sg] = ps if l[sg] is None else l[sg] + ps
                        p_ref[g, sg * NS + u, r0:r1, :] = p.astype(BF16)
                        if i == len(WCH) - 2:
                            m_ref[nset * g + sg, :, u * T:(u + 1) * T] = l[sg]
                return post

            return [lambda u0=u0, i=i: [run(u, i) for u in (u0, u0 + 1)]
                    for u0 in range(0, NS, 2) for i in range(len(WCH) - 1)]

        def pv_ops(g, b):
            acc = [None] * 8

            def run(sg, c):
                parts = []
                for u in range(NS):
                    lo = c * T - SQ * u
                    r0, r1 = max(lo, 0), min(lo + T, WIN + SQ)
                    pieces = []
                    if r0 > lo:
                        pieces.append(jnp.zeros(((r0 - lo) // 2, T), U32))
                    pieces.append(pltpu.bitcast(p_ref[g, sg * NS + u, r0:r1, :], U32))
                    if lo + T > r1:
                        pieces.append(jnp.zeros(((lo + T - r1) // 2, T), U32))
                    parts.append(jnp.concatenate(pieces, axis=0))
                vs = v_rows4(g, sg, b + c)
                for a0 in range(NS):
                    hh = sg * NS + a0
                    o = _dot(vs[a0], _bf(pick(parts, a0)))
                    acc[hh] = o if acc[hh] is None else acc[hh] + o
                if c == 2:
                    ls = m_ref[nset * g + sg]
                    ls = [ls[:, u * T:(u + 1) * T] for u in range(NS)]
                    outs = []
                    for a0 in range(NS):
                        o = acc[sg * NS + a0] * _recip(
                            jnp.sum(pick(ls, a0), axis=0, keepdims=True))
                        outs.append(pltpu.roll(o, T - SQ * a0, 1) if a0 else o)
                    oT_ref[g * T + sg * NS * DH:g * T + (sg + 1) * NS * DH,
                           pl.ds(_mul(b, T), T)] = jnp.concatenate(outs, axis=0).astype(BF16)

            return [lambda c=c, sg=sg: run(sg, c) for c in range(3) for sg in range(nset)]

        def body(bb, carry):
            npc = NWP // (NT // WQ)
            for i in range(npc):
                transpose_wb(bb * npc + i)
            for dq in range(WQ):
                b = bb * WQ + dq
                for g in range(NG):
                    qk = qk_ops(g, b, dq >= PT)
                    bp = b if g else (b - 1 if dq else jnp.maximum(b - 1, 0))
                    pv = pv_ops((g - 1) % NG, bp)
                    last = dq == WQ - 1 and g == NG - 1
                    for qk_p in qk:
                        for _ in range(min(2 if last else 1, len(pv))):
                            pv.pop(0)()
                        for post in qk_p():
                            post()
            return carry
        lax.fori_loop(0, NT // WQ, body, 0)
        for pv_p in pv_ops(NG - 1, NT - 1):
            pv_p()

    project(None, 0)
    for cp in wb_copies:
        cp.wait()

    def two_layers(it, carry):
        lax.cond(ok_ref[0] != 0, attn_window_fast, lambda: attn_max(True))
        project(0, 1)
        lax.cond(ok_ref[0] != 0, attn_full_fast, lambda: attn_max(False))
        pl.when(it == 0)(lambda: project(1, 0))
        return carry
    lax.fori_loop(0, 2, two_layers, 0)
    finish(1)


@jax.jit
def pallas_interleave_layers__sliding_block__mha_block__prompt_kernel(
    A_x: jax.Array,
    A_wqkv: jax.Array,
    A_wo: jax.Array,
    B_x: jax.Array,
    B_wqkv: jax.Array,
    B_wo: jax.Array,
):
    del B_x
    x = A_x.reshape(S, D)
    out = pl.pallas_call(
        _kernel,
        out_shape=jax.ShapeDtypeStruct((S, D), A_x.dtype),
        in_specs=[pl.BlockSpec(memory_space=pl.ANY)] * 5,
        out_specs=pl.BlockSpec(memory_space=pl.ANY),
        scratch_shapes=[
            pltpu.VMEM((S, D), BF16),
            pltpu.VMEM((3, D, D), BF16),
            pltpu.VMEM((D, 5 * D), BF16),
            pltpu.SemaphoreType.DMA((2 * NX + 6,)),
            pltpu.VMEM((D, S), F32),
            pltpu.VMEM((3 * D, D), BF16),
            pltpu.VMEM((5 * D, D), BF16),
            pltpu.VMEM((NT, NG, T // 2, T), U32),
            pltpu.VMEM((NG, (S + WIN) // 2, T), U32),
            pltpu.VMEM((NG, S // 2, T), U32),
            pltpu.VMEM((NT + PT, NG, T // 2, T), U32),
            pltpu.VMEM((D, S), BF16),
            pltpu.VMEM((S, 4 * T), F32),
            pltpu.VMEM((8, 8, 4 * T), F32),
            pltpu.VMEM((3, 3 * T, T), F32),
            pltpu.VMEM((2 * NS + 1, WIN + SQ, T), F32),
            pltpu.VMEM((NG, 8, 3 * T, T), BF16),
            pltpu.VMEM((2 * QB, 4 * DH, 8, T), F32),
            pltpu.VMEM((NPIECE, T, VK, T), F32),
            pltpu.VMEM((NPIECE, T, VK, T), F32),
            pltpu.VMEM((NG, NPIECE, VK, T), F32),
            pltpu.VMEM((NCARRY, T, 4 * T), F32),
            pltpu.VMEM((4, DH, T), F32),
            pltpu.VMEM((4, 8, HT), F32),
            pltpu.SMEM((1,), jnp.int32),
        ],
        compiler_params=pltpu.CompilerParams(vmem_limit_bytes=100 * 1024 * 1024),
        name="interleave_attn",
    )(x, A_wqkv, A_wo, B_wqkv, B_wo)
    return out.reshape(A_x.shape)
```

```python
import math

import jax
import jax.numpy as jnp
from jax import lax
import jax.experimental.pallas as pl
import jax.experimental.pallas.tpu as pltpu

S = 2048
D = 512
H = 32
DH = 16
WIN = 256
EPS = 1e-5

T = 128
NT = S // T
NG = D // T
PT = WIN // T
NEG = -1e30
QSCALE = (DH ** -0.5) * math.log2(math.e)
TT = 512
HT = TT // 2
NX = S // TT

SMAX = 60.0
VMAX = 2.0 ** 50
VMIN = 2.0 ** -40

QB = 2
VK = 16
PPC = TT // T + 1
NPIECE = NX * PPC
XSLOT = 1
EXTRA = ((13, 12, (5, 7, 9, 11)), (9, 11, (4, 6, 8, 10)))
DELAY = 9
NCARRY = 2
NS = 4
SQ = T // NS
WCH = (0, 96, 192, 288)
WQ = 4
NWP = 5 * D // T

F32 = jnp.float32
BF16 = jnp.bfloat16
U32 = jnp.uint32


def _dot(a, b):
    return jnp.dot(a, b, preferred_element_type=F32)


def _bf(x):
    return pltpu.bitcast(x, BF16)


def _pk(x):
    return pltpu.bitcast(x.astype(BF16), U32)


def _recip(x):
    r = pl.reciprocal(x, approx=True)
    return r * (2.0 - x * r)


def _mul(a, n):
    return a * n if isinstance(a, int) else pl.multiple_of(a * n, n)


def _kernel(x_hbm, awqkv_hbm, awo_hbm, bwqkv_hbm, bwo_hbm, out_hbm,
            x_ref, wa_ref, wb2_ref, sems, xT_ref, waT_ref, wbT_ref,
            qu, ku, khu, vu, oT_ref, s_ref, m_ref, bias_ref, wb_ref,
            p_ref, qb_ref, kb0_ref, kb1_ref, kf_ref, cp_ref, ca_ref, st_ref, ok_ref):
    kbs = (kb0_ref, kb1_ref)

    def x_copy(i):
        return pltpu.make_async_copy(x_hbm.at[pl.ds(i * HT, HT)],
                                     x_ref.at[pl.ds(i * HT, HT)], sems.at[i])

    def out_copy(i):
        return pltpu.make_async_copy(x_ref.at[pl.ds(i * HT, HT)],
                                     out_hbm.at[pl.ds(i * HT, HT)], sems.at[i])

    wa_copies = [pltpu.make_async_copy(awqkv_hbm.at[:, j * D:(j + 1) * D], wa_ref.at[j],
                                       sems.at[2 * NX + j]) for j in range(3)]
    wb_src = [awo_hbm] + [bwqkv_hbm.at[:, j * D:(j + 1) * D] for j in range(3)] + [bwo_hbm]
    wb_copies = [pltpu.make_async_copy(src, wb2_ref.at[j], sems.at[2 * NX + 3 + j])
                 for j, src in enumerate(wb_src)]

    def wqkv_t(li, j):
        return waT_ref[j * D:(j + 1) * D, :] if li == 0 else wbT_ref[(j + 1) * D:(j + 2) * D, :]

    def wo_t(li):
        return wbT_ref[0:D, :] if li == 0 else wbT_ref[4 * D:5 * D, :]

    def transpose_wb(piece):
        cols = pl.ds(_mul(lax.bitwise_and(piece, NG - 1), T), T)
        w = wb2_ref[lax.shift_right_logical(piece, 2), :, cols]
        wbT_ref[pl.ds(_mul(piece, T), T), :] = w.astype(F32).T.astype(BF16)

    x_copy(0).start()
    for cp in wa_copies:
        cp.start()
    x_copy(1).start()
    x_copy(2).start()
    for g in range(NG):
        ku[g, 0:WIN // 2, :] = jnp.zeros((WIN // 2, T), U32)
    for c in range(PT):
        vu[c] = jnp.zeros((NG, T // 2, T), U32)
    row = lax.broadcasted_iota(jnp.int32, (3 * T, T), 0)
    col = lax.broadcasted_iota(jnp.int32, (3 * T, T), 1)
    band = (row > col) & (row <= col + WIN)
    for v in range(3):
        bias_ref[v] = jnp.where(band & (row >= WIN - v * T), 0.0, NEG).astype(F32)
    row = lax.broadcasted_iota(jnp.int32, (WIN + SQ, T), 0)
    col = lax.broadcasted_iota(jnp.int32, (WIN + SQ, T), 1) % SQ
    band = (row > col) & (row <= col + WIN)
    for v in range(2 * NS + 1):
        wb_ref[v] = jnp.where(band & (row >= WIN - v * SQ), 0.0, NEG).astype(F32)
    p_ref[NG - 1] = jnp.zeros(p_ref.shape[1:], BF16)
    m_ref[...] = jnp.zeros(m_ref.shape, F32)
    cp_ref[...] = jnp.zeros(cp_ref.shape, F32)
    ca_ref[...] = jnp.zeros(ca_ref.shape, F32)
    oT_ref[...] = jnp.zeros(oT_ref.shape, BF16)

    def head_norm2(a):
        n2 = jnp.sum((a * a).reshape(H, DH, HT), axis=1)
        return jnp.max(n2.reshape(H // 8, 8, HT), axis=0)

    def residual(lo, h0):
        return xT_ref[:, pl.ds(h0, HT)] + _dot(wo_t(lo), oT_ref[:, pl.ds(h0, HT)])

    def normalize(lo, h0):
        if lo is None:
            x = x_ref[pl.ds(h0, HT), :].astype(F32).T
        else:
            x = residual(lo, h0)
        xT_ref[:, pl.ds(h0, HT)] = x
        mu = jnp.mean(x, axis=0, keepdims=True)
        xc = x - mu
        var = jnp.mean(xc * xc, axis=0, keepdims=True)
        return (xc * lax.rsqrt(var + EPS)).astype(BF16)

    def qkv(li, t, hf, xn, which):
        for w in which:
            qkv1(li, t, hf, xn, w)

    def qkv1(li, t, hf, xn, which):
        full = li == 1
        hh0 = _mul(t, TT // 2) + hf * (HT // 2)
        c0 = t * (TT // T) + hf * (HT // T)
        if which == 'k':
            kT = _dot(wqkv_t(li, 1), xn)
            st_ref[1] = jnp.maximum(st_ref[1], head_norm2(kT))
            kf = kT.T
            kk = kf.astype(BF16)
            for g in range(NG):
                ku[g, pl.ds(WIN // 2 + hh0, HT // 2), :] = _pk(kf[:, g * T:(g + 1) * T])
            if full:
                for g in range(NG):
                    khu[g, pl.ds(hh0, HT // 2), :] = _pk(
                        pltpu.roll(kf[:, g * T:(g + 1) * T], T // 2, 1))
                for c in range(HT // T):
                    cl = hf * (HT // T) + c
                    pieces = [(cl, c * T)]
                    if cl == XSLOT:
                        pieces.append((TT // T, c * T + VK))
                    for slot, r0 in pieces:
                        piece = t * PPC + slot
                        for g in range(NG):
                            kf_ref[g, piece] = kk[r0:r0 + VK, g * T:(g + 1) * T].astype(F32)
                        kp = kk[r0:r0 + VK, 0:T].astype(F32)
                        kb0_ref[piece] = jnp.stack(
                            [jnp.broadcast_to(kp[:, d:d + 1], (VK, T)) for d in range(T)])
        if which == 'q':
            q = _dot(wqkv_t(li, 0), xn) * QSCALE
            st_ref[0] = jnp.maximum(st_ref[0], head_norm2(q))
            for c in range(HT // T):
                qc = q[:, c * T:(c + 1) * T]
                if not full:
                    qc = jnp.concatenate(
                        [pltpu.roll(qc[DH * h:DH * (h + 1)], SQ * (h % NS), 1)
                         if h % NS else qc[DH * h:DH * (h + 1)] for h in range(H)], axis=0)
                for g in range(NG):
                    qu[c0 + c, g] = _pk(qc[g * T:(g + 1) * T])
        if which == 'v':
            v = _dot(wqkv_t(li, 2), xn)
            st_ref[2] = jnp.maximum(
                st_ref[2], jnp.max(jnp.abs(v).reshape(D // 8, 8, HT), axis=0))
            for c in range(HT // T):
                for g in range(NG):
                    vu[PT + c0 + c, g] = _pk(v[g * T:(g + 1) * T, c * T:(c + 1) * T])

    def project(lo, li):
        st_ref[...] = jnp.zeros(st_ref.shape, F32)
        if lo is None:
            x_copy(0).wait()
            first = normalize(None, 0)
            for j in range(3):
                wa_copies[j].wait()
                waT_ref[j * D:(j + 1) * D, :] = wa_ref[j].astype(F32).T.astype(BF16)

            def body(t, xn0):
                tn = jnp.minimum(t + 1, NX - 1)
                x_copy(2 * t + 1).wait()
                pl.when(t + 1 < NX)(lambda: x_copy(2 * tn).wait())

                @pl.when(t == 0)
                def _():
                    for i in range(3, 2 * NX):
                        x_copy(i).start()
                    for cp in wb_copies:
                        cp.start()
                xn1 = normalize(None, _mul(t, TT) + HT)
                qkv(li, t, 0, xn0, 'vqk')
                qkv(li, t, 1, xn1, 'kq')
                nxt = normalize(None, _mul(tn, TT))
                qkv(li, t, 1, xn1, 'v')
                return nxt
            lax.fori_loop(0, NX, body, first)
        else:
            def body(t, carry):
                xns = [normalize(lo, _mul(t, TT) + hf * HT) for hf in range(2)]
                for hf in range(2):
                    qkv(li, t, hf, xns[hf], 'kqv')
                return carry
            lax.fori_loop(0, NX, body, 0)
        qk2 = jnp.max(st_ref[0]) * jnp.max(st_ref[1])
        vm = jnp.max(st_ref[2])
        ok = (qk2 * 1.05 <= SMAX * SMAX) & (vm <= VMAX) & (vm >= VMIN)
        ok_ref[0] = ok.astype(jnp.int32)

    def finish(lo):
        def body(t, carry):
            for hf in range(4):
                i = 4 * t + hf
                x_ref[pl.ds(_mul(i, HT), HT), :] = residual(lo, _mul(i, HT)).T.astype(BF16)
                out_copy(i).start()
            return carry
        lax.fori_loop(0, S // (4 * HT), body, 0)
        for i in range(S // HT):
            out_copy(i).wait()

    def q_weights(g, heads, qi, rotated=False, base=0):
        cols = []
        for hh in heads:
            parts = []
            if hh > base:
                parts.append(jnp.zeros((8 * (hh - base), T), U32))
            slab = qu[qi, g, 8 * hh:8 * (hh + 1), :]
            if rotated and hh % NS:
                slab = pltpu.roll(slab, T - SQ * (hh % NS), 1)
            parts.append(slab)
            if hh - base < 7:
                parts.append(jnp.zeros((8 * (7 - hh + base), T), U32))
            cols.append(jnp.concatenate(parts, axis=0))
        return _bf(jnp.concatenate(cols, axis=1))

    def v_rows(g, hh, kt):
        return _bf(vu[kt, g, 8 * hh:8 * (hh + 1), :])

    def v_rows4(g, half, kt):
        vv = vu[kt, g, 32 * half:32 * (half + 1), :]
        return [_bf(vv[8 * j:8 * (j + 1)]) for j in range(4)]

    def store_o(g, hh, qi, val):
        oT_ref[pl.ds(_mul(g, T) + DH * hh, DH), pl.ds(_mul(qi, T), T)] = val.astype(BF16)

    def attend_max(g, q, k0, nc, ct, bias):
        ck = ct * T
        for half in range(2):
            heads = range(4 * half, 4 * half + 4)
            w = q_weights(g, heads, q, rotated=bias is not None)

            def scores(i, m):
                sc = _dot(_bf(ku[g, pl.ds(_mul(k0 + i * ct, T // 2), ck // 2), :]), w)
                if bias is not None:
                    sc = sc + jnp.concatenate([bias[...]] * 4, axis=1)
                s_ref[pl.ds(_mul(i, ck), ck), :] = sc
                return jnp.maximum(m, jnp.max(sc.reshape(ck // 8, 8, 4 * T), axis=0))
            m = lax.fori_loop(0, nc, scores, jnp.full((8, 4 * T), -jnp.inf, F32))
            m = jnp.max(m, axis=0, keepdims=True)

            def weigh(i, carry):
                l, acc = carry
                p = jnp.exp2(s_ref[pl.ds(_mul(i, ck), ck), :] - m)
                l = l + jnp.sum(p.reshape(ck // 8, 8, 4 * T), axis=0)
                acc = list(acc)
                for j, hh in enumerate(heads):
                    for c in range(ct):
                        acc[j] = acc[j] + _dot(
                            v_rows(g, hh, k0 + i * ct + c),
                            p[c * T:(c + 1) * T, j * T:(j + 1) * T].astype(BF16))
                return l, tuple(acc)
            l, acc = lax.fori_loop(
                0, nc, weigh,
                (jnp.zeros((8, 4 * T), F32), (jnp.zeros((DH, T), F32),) * 4))
            linv = 1.0 / jnp.sum(l, axis=0, keepdims=True)
            for j, hh in enumerate(heads):
                store_o(g, hh, q, acc[j] * linv[:, j * T:(j + 1) * T])

    def attn_max(window):
        def body(b, carry):
            g = lax.shift_right_logical(b, 4)
            q = lax.bitwise_and(b, NT - 1)
            if window:
                attend_max(g, q, q, 1, 3, bias_ref.at[jnp.minimum(q, 2)])
            else:
                attend_max(g, q, PT, NT // 4, 4, None)
            return carry
        lax.fori_loop(0, NG * NT, body, 0)
        if window:
            def tr(piece, carry):
                transpose_wb(piece)
                return carry
            lax.fori_loop(0, NWP, tr, 0)

    carry_acc = [None] * 4

    def finalize(item, acc, l):
        g, half, q = item
        linv = _recip(jnp.sum(l, axis=0, keepdims=True))
        o = jnp.concatenate([acc[j] * linv[:, j * T:(j + 1) * T] for j in range(4)], axis=0)
        oT_ref[pl.ds(_mul(g, T) + 4 * DH * half, 4 * DH), pl.ds(_mul(q, T), T)] = o.astype(BF16)

    def finish_carry(item, i):
        vs = v_rows4(item[0], item[1], PT + NT - NCARRY + i)
        for j in range(4):
            o = _dot(vs[j], cp_ref[i, :, j * T:(j + 1) * T])
            carry_acc[j] = (ca_ref[j] if i == 0 else carry_acc[j]) + o
        if i == NCARRY - 1:
            finalize(item, carry_acc, m_ref[0])

    def build_qb(item, slot, step):
        g, half, q = item
        hh = 4 * half + step // 4
        qs = _bf(qu[q, g, 8 * hh:8 * (hh + 1), :]).astype(F32)
        qb_ref[slot, 4 * step:4 * step + 4] = jnp.stack(
            [jnp.broadcast_to(qs[r % DH:r % DH + 1, :], (8, T))
             for r in range(4 * step, 4 * step + 4)])

    def block_full(items, prev_item, next_items, blk, par):
        g = items[0][0]
        kb = kbs[par]
        gn = jnp.minimum(g + 1, NG - 1)
        n_items = len(items)
        ngr = T // 16
        piece = lambda c: (c // (TT // T)) * PPC + c % (TT // T)
        spare = lambda c: (c // (TT // T)) * PPC + TT // T
        order = [None] * NT
        for xt, pos, _ in EXTRA:
            order[pos] = xt
        use = {c: [piece(c), spare(c)] if c in order else [piece(c)] for c in range(NT)}
        rest = [c for c in range(NT) if c not in order]
        order = [c if c is not None else rest.pop(0) for c in order]
        tiles = [(u, c) for u in range(n_items) for c in order]
        stream = [(u, c, gr) for (u, c) in tiles
                  for gr in range(ngr - 1, len(use[c]) - 1, -1)]
        end = {(u, c): n + 1 for n, (u, c, _) in enumerate(stream)}
        slots = {end[tiles[0]] + DELAY - (NCARRY - i) * (ngr - 1): i for i in range(NCARRY)}
        for t in tiles[:len(tiles) - NCARRY]:
            slots[end[t] + DELAY] = t
        cuts = sorted(set(slots) | {end[(u, NT - 1)] for u in range(n_items)})
        release = [[(u, j, piece(c)) for j in range(4)] for (u, c) in tiles]
        for u in range(n_items):
            for xt, _, rel in EXTRA:
                for j in range(4):
                    release[u * NT + rel[j]].append((u, j, spare(xt)))
        spl = len(tiles) * (NT // QB) // T
        ws, sres, l, acc, probs, vres = {}, {}, {}, {}, {}, {}
        always = jnp.full((8, T), ok_ref[0], jnp.int32) != 0
        lastdep, lastbuilt, lastextra = None, [], []

        def vpu_scores(u, j, pc, dep):
            hh = 4 * items[u][1] + j
            kv = kb[pc, DH * hh:DH * (hh + 1)].reshape(DH, VK // 8, 8, T)
            qv = qb_ref[u, DH * j:DH * (j + 1)]
            if dep is not None:
                qv = jnp.concatenate(
                    [jnp.where(always[None], qv[0:1], dep[None]), qv[1:]], axis=0)
            return jnp.sum(kv * qv[:, None], axis=0).reshape(VK, T)

        def do_pv(u, c):
            p = probs.pop((u, c))
            vs = v_rows4(g, items[u][1], PT + c)
            for j in range(4):
                o = _dot(vs[j], p[:, j * T:(j + 1) * T])
                acc[(u, j)] = o if c == 0 else acc[(u, j)] + o
            if c == NT - 1:
                finalize(items[u], [acc[(u, j)] for j in range(4)], l[u])

        x = 0
        for y in cuts:
            ch = stream[x:y]
            x = y
            u = ch[0][0]
            _, half, q = items[u]
            if u not in ws:
                ws[u] = q_weights(g, range(4 * half, 4 * half + 4), q, base=4 * half)
            ksrc, koff = (khu, 0) if half else (ku, PT)
            rows = []
            for c in dict.fromkeys(c for (_, c, _) in ch):
                grs = [gr for (_, cc, gr) in ch if cc == c]
                r0 = (koff + c) * (T // 2) + 8 * grs[-1]
                kt = ksrc[g, r0:r0 + 8 * len(grs), :]
                rows += [kt[8 * (gr - grs[-1]):8 * (gr - grs[-1] + 1)] for gr in grs]
            lhs = jnp.concatenate(rows, axis=0)
            sc = _dot(_bf(lhs), ws[u])
            if y in slots:
                if isinstance(slots[y], int):
                    finish_carry(prev_item, slots[y])
                else:
                    do_pv(*slots[y])
            n0 = 0
            for c in dict.fromkeys(c for (_, c, _) in ch):
                cnt = sum(cc == c for (_, cc, _) in ch)
                sres.setdefault((u, c), []).append(sc[16 * n0:16 * (n0 + cnt)])
                n0 += cnt
            for (_, c, gr) in ch:
                nv = len(use[c])
                if gr != nv:
                    continue
                n = tiles.index((u, c))
                st = jnp.concatenate(sres.pop((u, c)), axis=0)
                d = blk * (len(tiles) // spl) + n // spl
                pa = (n % spl) * PPC
                pb = pa + PPC - (pa + PPC - 1 not in [spare(xt) for xt, _, _ in EXTRA])
                src = kf_ref[gn, pa:pb].reshape((pb - pa) * VK, T)
                colv = jnp.take_along_axis(
                    src, jnp.full(src.shape, d, jnp.int32), axis=1, mode="promise_in_bounds")
                kbs[1 - par][pa:pb, d] = colv.reshape(pb - pa, VK, T)
                built = colv
                if u < 2:
                    build_qb(items[n_items - 2 + u], n_items - 2 + u, n % NT)
                else:
                    build_qb(next_items[u - 2], u - 2, n % NT)
                todo = release[n]
                for e, unit in enumerate(todo):
                    dep = None
                    if lastdep is not None:
                        nr = lastdep.shape[0] // 8
                        rr = ((e * nr) // len(todo)) ^ 1
                        dep = jnp.maximum(lastdep[rr * 8:(rr + 1) * 8, 0:T],
                                          lastbuilt[e * 8:(e + 1) * 8])
                        if e == 0:
                            for xr in lastextra:
                                dep = jnp.maximum(dep, jnp.maximum(xr[0:8], xr[8:16]))
                    vres[unit] = vpu_scores(*unit, dep)
                lastextra = [vres[unit] for unit in todo[4:]]
                parts = [jnp.concatenate([vres.pop((u, j, pc)) for j in range(4)], axis=1)
                         for pc in reversed(use[c])]
                p = jnp.exp2(jnp.concatenate([st] + parts, axis=0))
                if c == 0:
                    l[u] = jnp.sum(p.reshape(T // 8, 8, 4 * T), axis=0)
                else:
                    l[u] = jnp.sum(jnp.concatenate([l[u], p], axis=0).reshape(
                        T // 8 + 1, 8, 4 * T), axis=0)
                p = jnp.concatenate(
                    [p[16 * gg:16 * (gg + 1)] for gg in range(ngr - 1, -1, -1)], axis=0)
                if n >= len(tiles) - NCARRY:
                    cp_ref[n - (len(tiles) - NCARRY)] = p
                else:
                    probs[(u, c)] = p
                lastdep, lastbuilt = st, built
        ca_ref[...] = jnp.stack([acc[(n_items - 1, j)] for j in range(4)])
        m_ref[0] = l[n_items - 1]

    def attn_full_fast():
        nb = NT // QB

        def items(g, blk):
            return [(g, half, blk * QB + dq) for dq in range(QB) for half in range(2)]

        def items_at(b):
            return items(lax.shift_right_logical(b, nb.bit_length() - 1),
                         lax.bitwise_and(b, nb - 1))

        for u, item in enumerate(items(0, 0)[:-2]):
            for step in range(NT):
                build_qb(item, u, step)

        def outer(gp, carry):
            for par in range(2):
                g = 2 * gp + par

                def body(blk, c2, g=g, par=par):
                    prev = items_at(jnp.maximum(g * nb + blk - 1, 0))[-1]
                    nxt = items_at(jnp.minimum(g * nb + blk + 1, NG * nb - 1))
                    block_full(items(g, blk), prev, nxt, blk, par)
                    return c2
                lax.fori_loop(0, nb, body, 0)
            return carry
        lax.fori_loop(0, NG // 2, outer, 0)
        for i in range(NCARRY):
            finish_carry(items(NG - 1, nb - 1)[-1], i)

    def attn_window_fast():
        nset = 8 // NS

        is_grp = {(rows, a): lax.broadcasted_iota(jnp.int32, (rows, T), 1) // SQ == a
                  for rows in (8, T // 2) for a in range(NS)}

        def pick(parts, a0):
            out = parts[0]
            for u in range(1, NS):
                out = jnp.where(is_grp[(out.shape[0], (a0 + u) % NS)], parts[u], out)
            return out

        def qk_ops(g, b, interior):
            qg = qu[b, g]
            slabs = [qg[8 * hh:8 * (hh + 1)] for hh in range(8)]
            zero = jnp.zeros((8, T), U32)
            state = {}

            def run(u, i):
                if i == 0:
                    tiles = [jnp.concatenate(
                        [jnp.where(is_grp[(8, (hh % NS + u) % NS)], slabs[hh], zero)
                         if hh // NS == sg else zero for hh in range(8)], axis=0)
                        for sg in range(nset)]
                    state[u] = (_bf(jnp.concatenate(tiles, axis=1)), [None] * nset)
                w, l = state[u]
                r0, r1 = WCH[i], WCH[i + 1]
                kwin = ku.at[g, pl.ds(_mul(b, T // 2), 3 * T // 2)]
                sc = _dot(_bf(kwin[(SQ * u + r0) // 2:(SQ * u + r1) // 2, :]), w)

                def post():
                    m0 = max(r0, WIN) if interior and r0 >= SQ else r0
                    m1 = min(r1, SQ) if interior and r1 <= WIN else r1
                    if m1 > m0:
                        bias = wb_ref[jnp.minimum(NS * b + u, 2 * NS), m0:m1, :]
                    for sg in range(nset):
                        z = sc[:, sg * T:(sg + 1) * T]
                        if m1 > m0:
                            z = jnp.concatenate(
                                [e for e in (z[:m0 - r0], z[m0 - r0:m1 - r0] + bias, z[m1 - r0:])
                                 if e.shape[0]], axis=0)
                        p = jnp.exp2(z)
                        ps = jnp.sum(p.reshape((r1 - r0) // 8, 8, T), axis=0)
                        l[sg] = ps if l[sg] is None else l[sg] + ps
                        p_ref[g, sg * NS + u, r0:r1, :] = p.astype(BF16)
                        if i == len(WCH) - 2:
                            m_ref[nset * g + sg, :, u * T:(u + 1) * T] = l[sg]
                return post

            return [lambda u0=u0, i=i: [run(u, i) for u in (u0, u0 + 1)]
                    for u0 in range(0, NS, 2) for i in range(len(WCH) - 1)]

        def pv_ops(g, b):
            acc = [None] * 8

            def run(sg, c):
                parts = []
                for u in range(NS):
                    lo = c * T - SQ * u
                    r0, r1 = max(lo, 0), min(lo + T, WIN + SQ)
                    pieces = []
                    if r0 > lo:
                        pieces.append(jnp.zeros(((r0 - lo) // 2, T), U32))
                    pieces.append(pltpu.bitcast(p_ref[g, sg * NS + u, r0:r1, :], U32))
                    if lo + T > r1:
                        pieces.append(jnp.zeros(((lo + T - r1) // 2, T), U32))
                    parts.append(jnp.concatenate(pieces, axis=0))
                vs = v_rows4(g, sg, b + c)
                for a0 in range(NS):
                    hh = sg * NS + a0
                    o = _dot(vs[a0], _bf(pick(parts, a0)))
                    acc[hh] = o if acc[hh] is None else acc[hh] + o
                if c == 2:
                    ls = m_ref[nset * g + sg]
                    ls = [ls[:, u * T:(u + 1) * T] for u in range(NS)]
                    outs = []
                    for a0 in range(NS):
                        o = acc[sg * NS + a0] * _recip(
                            jnp.sum(pick(ls, a0), axis=0, keepdims=True))
                        outs.append(pltpu.roll(o, T - SQ * a0, 1) if a0 else o)
                    oT_ref[g * T + sg * NS * DH:g * T + (sg + 1) * NS * DH,
                           pl.ds(_mul(b, T), T)] = jnp.concatenate(outs, axis=0).astype(BF16)

            return [lambda c=c, sg=sg: run(sg, c) for c in range(3) for sg in range(nset)]

        def body(bb, carry):
            npc = NWP // (NT // WQ)
            for i in range(npc):
                transpose_wb(bb * npc + i)
            for dq in range(WQ):
                b = bb * WQ + dq
                for g in range(NG):
                    qk = qk_ops(g, b, dq >= PT)
                    bp = b if g else (b - 1 if dq else jnp.maximum(b - 1, 0))
                    pv = pv_ops((g - 1) % NG, bp)
                    last = dq == WQ - 1 and g == NG - 1
                    for qk_p in qk:
                        for _ in range(min(2 if last else 1, len(pv))):
                            pv.pop(0)()
                        for post in qk_p():
                            post()
            return carry
        lax.fori_loop(0, NT // WQ, body, 0)
        for pv_p in pv_ops(NG - 1, NT - 1):
            pv_p()

    project(None, 0)
    for cp in wb_copies:
        cp.wait()

    def two_layers(it, carry):
        lax.cond(ok_ref[0] != 0, attn_window_fast, lambda: attn_max(True))
        project(0, 1)
        lax.cond(ok_ref[0] != 0, attn_full_fast, lambda: attn_max(False))
        pl.when(it == 0)(lambda: project(1, 0))
        return carry
    lax.fori_loop(0, 2, two_layers, 0)
    finish(1)


@jax.jit
def pallas_interleave_layers__sliding_block__mha_block__prompt_kernel(
    A_x: jax.Array,
    A_wqkv: jax.Array,
    A_wo: jax.Array,
    B_x: jax.Array,
    B_wqkv: jax.Array,
    B_wo: jax.Array,
):
    del B_x
    x = A_x.reshape(S, D)
    out = pl.pallas_call(
        _kernel,
        out_shape=jax.ShapeDtypeStruct((S, D), A_x.dtype),
        in_specs=[pl.BlockSpec(memory_space=pl.ANY)] * 5,
        out_specs=pl.BlockSpec(memory_space=pl.ANY),
        scratch_shapes=[
            pltpu.VMEM((S, D), BF16),
            pltpu.VMEM((3, D, D), BF16),
            pltpu.VMEM((5, D, D), BF16),
            pltpu.SemaphoreType.DMA((2 * NX + 8,)),
            pltpu.VMEM((D, S), F32),
            pltpu.VMEM((3 * D, D), BF16),
            pltpu.VMEM((5 * D, D), BF16),
            pltpu.VMEM((NT, NG, T // 2, T), U32),
            pltpu.VMEM((NG, (S + WIN) // 2, T), U32),
            pltpu.VMEM((NG, S // 2, T), U32),
            pltpu.VMEM((NT + PT, NG, T // 2, T), U32),
            pltpu.VMEM((D, S), BF16),
            pltpu.VMEM((S, 4 * T), F32),
            pltpu.VMEM((8, 8, 4 * T), F32),
            pltpu.VMEM((3, 3 * T, T), F32),
            pltpu.VMEM((2 * NS + 1, WIN + SQ, T), F32),
            pltpu.VMEM((NG, 8, 3 * T, T), BF16),
            pltpu.VMEM((2 * QB, 4 * DH, 8, T), F32),
            pltpu.VMEM((NPIECE, T, VK, T), F32),
            pltpu.VMEM((NPIECE, T, VK, T), F32),
            pltpu.VMEM((NG, NPIECE, VK, T), F32),
            pltpu.VMEM((NCARRY, T, 4 * T), F32),
            pltpu.VMEM((4, DH, T), F32),
            pltpu.VMEM((4, 8, HT), F32),
            pltpu.SMEM((1,), jnp.int32),
        ],
        compiler_params=pltpu.CompilerParams(vmem_limit_bytes=100 * 1024 * 1024),
        name="interleave_attn",
    )(x, A_wqkv, A_wo, B_wqkv, B_wo)
    return out.reshape(A_x.shape)
```

```python
import math

import jax
import jax.numpy as jnp
from jax import lax
import jax.experimental.pallas as pl
import jax.experimental.pallas.tpu as pltpu

S = 2048
D = 512
H = 32
DH = 16
WIN = 256
EPS = 1e-5

T = 128
NT = S // T
NG = D // T
PT = WIN // T
NEG = -1e30
QSCALE = (DH ** -0.5) * math.log2(math.e)
TT = 512
HT = TT // 2
NX = S // TT

SMAX = 60.0
VMAX = 2.0 ** 50
VMIN = 2.0 ** -40

QB = 2
VK = 16
PPC = TT // T + 1
NPIECE = NX * PPC
XSLOT = 1
EXTRA = ((13, 13, (2, 5, 8, 11)), (9, 12, (1, 4, 7, 10)), (5, 11, (0, 3, 6, 9)))
DELAY = 9
NCARRY = 2
NS = 8
SQ = T // NS
WCH = (0, 96, 192, WIN + SQ)
WQ = 4
NWP = 5 * D // T

F32 = jnp.float32
BF16 = jnp.bfloat16
U32 = jnp.uint32


def _dot(a, b):
    return jnp.dot(a, b, preferred_element_type=F32)


def _bf(x):
    return pltpu.bitcast(x, BF16)


def _pk(x):
    return pltpu.bitcast(x.astype(BF16), U32)


def _recip(x):
    r = pl.reciprocal(x, approx=True)
    return r * (2.0 - x * r)


def _mul(a, n):
    return a * n if isinstance(a, int) else pl.multiple_of(a * n, n)


def _kernel(x_hbm, awqkv_hbm, awo_hbm, bwqkv_hbm, bwo_hbm, out_hbm,
            x_ref, wa_ref, wb2_ref, sems, xT_ref, waT_ref, wbT_ref,
            qu, ku, khu, vu, oT_ref, s_ref, m_ref, bias_ref, wb_ref,
            p_ref, qb_ref, kb0_ref, kb1_ref, kf_ref, cp_ref, ca_ref, st_ref, ok_ref):
    kbs = (kb0_ref, kb1_ref)

    def x_copy(i):
        return pltpu.make_async_copy(x_hbm.at[pl.ds(i * HT, HT)],
                                     x_ref.at[pl.ds(i * HT, HT)], sems.at[i])

    def out_copy(i):
        return pltpu.make_async_copy(x_ref.at[pl.ds(i * HT, HT)],
                                     out_hbm.at[pl.ds(i * HT, HT)], sems.at[i])

    wa_copies = [pltpu.make_async_copy(awqkv_hbm.at[:, j * D:(j + 1) * D], wa_ref.at[j],
                                       sems.at[2 * NX + j]) for j in range(3)]
    wb_src = [awo_hbm] + [bwqkv_hbm.at[:, j * D:(j + 1) * D] for j in range(3)] + [bwo_hbm]
    wb_copies = [pltpu.make_async_copy(src, wb2_ref.at[j], sems.at[2 * NX + 3 + j])
                 for j, src in enumerate(wb_src)]

    def wqkv_t(li, j):
        return waT_ref[j * D:(j + 1) * D, :] if li == 0 else wbT_ref[(j + 1) * D:(j + 2) * D, :]

    def wo_t(li):
        return wbT_ref[0:D, :] if li == 0 else wbT_ref[4 * D:5 * D, :]

    def transpose_wb(piece):
        cols = pl.ds(_mul(lax.bitwise_and(piece, NG - 1), T), T)
        w = wb2_ref[lax.shift_right_logical(piece, 2), :, cols]
        wbT_ref[pl.ds(_mul(piece, T), T), :] = w.astype(F32).T.astype(BF16)

    x_copy(0).start()
    for cp in wa_copies:
        cp.start()
    x_copy(1).start()
    x_copy(2).start()
    for g in range(NG):
        ku[g, 0:WIN // 2, :] = jnp.zeros((WIN // 2, T), U32)
    for c in range(PT):
        vu[c] = jnp.zeros((NG, T // 2, T), U32)
    row = lax.broadcasted_iota(jnp.int32, (3 * T, T), 0)
    col = lax.broadcasted_iota(jnp.int32, (3 * T, T), 1)
    band = (row > col) & (row <= col + WIN)
    for v in range(3):
        bias_ref[v] = jnp.where(band & (row >= WIN - v * T), 0.0, NEG).astype(F32)
    row = lax.broadcasted_iota(jnp.int32, (WIN + SQ, T), 0)
    col = lax.broadcasted_iota(jnp.int32, (WIN + SQ, T), 1) % SQ
    band = (row > col) & (row <= col + WIN)
    for v in range(2 * NS + 1):
        wb_ref[v, 0:WIN + SQ] = jnp.where(
            band & (row >= WIN - v * SQ), 0.0, NEG).astype(F32)
    p_ref[NG - 1] = jnp.zeros(p_ref.shape[1:], BF16)
    m_ref[...] = jnp.zeros(m_ref.shape, F32)
    cp_ref[...] = jnp.zeros(cp_ref.shape, F32)
    ca_ref[...] = jnp.zeros(ca_ref.shape, F32)
    oT_ref[...] = jnp.zeros(oT_ref.shape, BF16)

    def head_norm2(a):
        n2 = jnp.sum((a * a).reshape(H, DH, HT), axis=1)
        return jnp.max(n2.reshape(H // 8, 8, HT), axis=0)

    def residual(lo, h0):
        return xT_ref[:, pl.ds(h0, HT)] + _dot(wo_t(lo), oT_ref[:, pl.ds(h0, HT)])

    def normalize(lo, h0):
        if lo is None:
            x = x_ref[pl.ds(h0, HT), :].astype(F32).T
        else:
            x = residual(lo, h0)
        xT_ref[:, pl.ds(h0, HT)] = x
        mu = jnp.mean(x, axis=0, keepdims=True)
        xc = x - mu
        var = jnp.mean(xc * xc, axis=0, keepdims=True)
        return (xc * lax.rsqrt(var + EPS)).astype(BF16)

    def qkv(li, t, hf, xn, which):
        for w in which:
            qkv1(li, t, hf, xn, w)

    def qkv1(li, t, hf, xn, which):
        full = li == 1
        hh0 = _mul(t, TT // 2) + hf * (HT // 2)
        c0 = t * (TT // T) + hf * (HT // T)
        if which == 'k':
            kT = _dot(wqkv_t(li, 1), xn)
            st_ref[1] = jnp.maximum(st_ref[1], head_norm2(kT))
            kf = kT.T
            kk = kf.astype(BF16)
            for g in range(NG):
                ku[g, pl.ds(WIN // 2 + hh0, HT // 2), :] = _pk(kf[:, g * T:(g + 1) * T])
            if full:
                for g in range(NG):
                    khu[g, pl.ds(hh0, HT // 2), :] = _pk(
                        pltpu.roll(kf[:, g * T:(g + 1) * T], T // 2, 1))
                for c in range(HT // T):
                    cl = hf * (HT // T) + c
                    pieces = [(cl, c * T)]
                    if cl == XSLOT:
                        pieces.append((TT // T, c * T + VK))
                    for slot, r0 in pieces:
                        piece = t * PPC + slot
                        for g in range(NG):
                            kf_ref[g, piece] = kk[r0:r0 + VK, g * T:(g + 1) * T].astype(F32)
                        kp = kk[r0:r0 + VK, 0:T].astype(F32)
                        kb0_ref[piece] = jnp.stack(
                            [jnp.broadcast_to(kp[:, d:d + 1], (VK, T)) for d in range(T)])
        if which == 'q':
            q = _dot(wqkv_t(li, 0), xn) * QSCALE
            st_ref[0] = jnp.maximum(st_ref[0], head_norm2(q))
            for c in range(HT // T):
                qc = q[:, c * T:(c + 1) * T]
                if not full:
                    qc = jnp.concatenate(
                        [pltpu.roll(qc[DH * h:DH * (h + 1)], SQ * (h % NS), 1)
                         if h % NS else qc[DH * h:DH * (h + 1)] for h in range(H)], axis=0)
                for g in range(NG):
                    qu[c0 + c, g] = _pk(qc[g * T:(g + 1) * T])
        if which == 'v':
            v = _dot(wqkv_t(li, 2), xn)
            st_ref[2] = jnp.maximum(
                st_ref[2], jnp.max(jnp.abs(v).reshape(D // 8, 8, HT), axis=0))
            for c in range(HT // T):
                for g in range(NG):
                    vu[PT + c0 + c, g] = _pk(v[g * T:(g + 1) * T, c * T:(c + 1) * T])

    def project(lo, li):
        st_ref[...] = jnp.zeros(st_ref.shape, F32)
        if lo is None:
            x_copy(0).wait()
            first = normalize(None, 0)
            for j in range(3):
                wa_copies[j].wait()
                waT_ref[j * D:(j + 1) * D, :] = wa_ref[j].astype(F32).T.astype(BF16)

            def body(t, xn0):
                tn = jnp.minimum(t + 1, NX - 1)
                x_copy(2 * t + 1).wait()
                pl.when(t + 1 < NX)(lambda: x_copy(2 * tn).wait())

                @pl.when(t == 0)
                def _():
                    for i in range(3, 2 * NX):
                        x_copy(i).start()
                    for cp in wb_copies:
                        cp.start()
                xn1 = normalize(None, _mul(t, TT) + HT)
                qkv(li, t, 0, xn0, 'vqk')
                qkv(li, t, 1, xn1, 'kq')
                nxt = normalize(None, _mul(tn, TT))
                qkv(li, t, 1, xn1, 'v')
                return nxt
            lax.fori_loop(0, NX, body, first)
        else:
            def body(t, carry):
                xns = [normalize(lo, _mul(t, TT) + hf * HT) for hf in range(2)]
                for hf in range(2):
                    qkv(li, t, hf, xns[hf], 'kqv')
                return carry
            lax.fori_loop(0, NX, body, 0)
        qk2 = jnp.max(st_ref[0]) * jnp.max(st_ref[1])
        vm = jnp.max(st_ref[2])
        ok = (qk2 * 1.05 <= SMAX * SMAX) & (vm <= VMAX) & (vm >= VMIN)
        ok_ref[0] = ok.astype(jnp.int32)

    def finish(lo):
        def body(t, carry):
            for hf in range(4):
                i = 4 * t + hf
                x_ref[pl.ds(_mul(i, HT), HT), :] = residual(lo, _mul(i, HT)).T.astype(BF16)
                out_copy(i).start()
            return carry
        lax.fori_loop(0, S // (4 * HT), body, 0)
        for i in range(S // HT):
            out_copy(i).wait()

    def q_weights(g, heads, qi, rotated=False, base=0):
        cols = []
        for hh in heads:
            parts = []
            if hh > base:
                parts.append(jnp.zeros((8 * (hh - base), T), U32))
            slab = qu[qi, g, 8 * hh:8 * (hh + 1), :]
            if rotated and hh % NS:
                slab = pltpu.roll(slab, T - SQ * (hh % NS), 1)
            parts.append(slab)
            if hh - base < 7:
                parts.append(jnp.zeros((8 * (7 - hh + base), T), U32))
            cols.append(jnp.concatenate(parts, axis=0))
        return _bf(jnp.concatenate(cols, axis=1))

    def v_rows(g, hh, kt):
        return _bf(vu[kt, g, 8 * hh:8 * (hh + 1), :])

    def v_rows4(g, half, kt):
        vv = vu[kt, g, 32 * half:32 * (half + 1), :]
        return [_bf(vv[8 * j:8 * (j + 1)]) for j in range(4)]

    def store_o(g, hh, qi, val):
        oT_ref[pl.ds(_mul(g, T) + DH * hh, DH), pl.ds(_mul(qi, T), T)] = val.astype(BF16)

    def attend_max(g, q, k0, nc, ct, bias):
        ck = ct * T
        for half in range(2):
            heads = range(4 * half, 4 * half + 4)
            w = q_weights(g, heads, q, rotated=bias is not None)

            def scores(i, m):
                sc = _dot(_bf(ku[g, pl.ds(_mul(k0 + i * ct, T // 2), ck // 2), :]), w)
                if bias is not None:
                    sc = sc + jnp.concatenate([bias[...]] * 4, axis=1)
                s_ref[pl.ds(_mul(i, ck), ck), :] = sc
                return jnp.maximum(m, jnp.max(sc.reshape(ck // 8, 8, 4 * T), axis=0))
            m = lax.fori_loop(0, nc, scores, jnp.full((8, 4 * T), -jnp.inf, F32))
            m = jnp.max(m, axis=0, keepdims=True)

            def weigh(i, carry):
                l, acc = carry
                p = jnp.exp2(s_ref[pl.ds(_mul(i, ck), ck), :] - m)
                l = l + jnp.sum(p.reshape(ck // 8, 8, 4 * T), axis=0)
                acc = list(acc)
                for j, hh in enumerate(heads):
                    for c in range(ct):
                        acc[j] = acc[j] + _dot(
                            v_rows(g, hh, k0 + i * ct + c),
                            p[c * T:(c + 1) * T, j * T:(j + 1) * T].astype(BF16))
                return l, tuple(acc)
            l, acc = lax.fori_loop(
                0, nc, weigh,
                (jnp.zeros((8, 4 * T), F32), (jnp.zeros((DH, T), F32),) * 4))
            linv = 1.0 / jnp.sum(l, axis=0, keepdims=True)
            for j, hh in enumerate(heads):
                store_o(g, hh, q, acc[j] * linv[:, j * T:(j + 1) * T])

    def attn_max(window):
        def body(b, carry):
            g = lax.shift_right_logical(b, 4)
            q = lax.bitwise_and(b, NT - 1)
            if window:
                attend_max(g, q, q, 1, 3, bias_ref.at[jnp.minimum(q, 2)])
            else:
                attend_max(g, q, PT, NT // 4, 4, None)
            return carry
        lax.fori_loop(0, NG * NT, body, 0)
        if window:
            def tr(piece, carry):
                transpose_wb(piece)
                return carry
            lax.fori_loop(0, NWP, tr, 0)

    carry_acc = [None] * 4

    def opaque_zero():
        return (jnp.full((DH, T), ok_ref[0], jnp.int32) - 1).astype(F32)

    def finalize(item, acc, l):
        g, half, q = item
        linv = _recip(jnp.sum(l, axis=0, keepdims=True))
        o = jnp.concatenate([acc[j] * linv[:, j * T:(j + 1) * T] for j in range(4)], axis=0)
        oT_ref[pl.ds(_mul(g, T) + 4 * DH * half, 4 * DH), pl.ds(_mul(q, T), T)] = o.astype(BF16)

    def finish_carry(item, i):
        vs = v_rows4(item[0], item[1], PT + NT - NCARRY + i)
        for j in range(4):
            o = _dot(vs[j], cp_ref[i, :, j * T:(j + 1) * T])
            carry_acc[j] = (ca_ref[j] if i == 0 else carry_acc[j]) + o
        if i == NCARRY - 1:
            finalize(item, carry_acc, m_ref[0])

    def build_qb(item, slot, step):
        g, half, q = item
        hh = 4 * half + step // 4
        qs = _bf(qu[q, g, 8 * hh:8 * (hh + 1), :]).astype(F32)
        qb_ref[slot, 4 * step:4 * step + 4] = jnp.stack(
            [jnp.broadcast_to(qs[r % DH:r % DH + 1, :], (8, T))
             for r in range(4 * step, 4 * step + 4)])

    def block_full(items, prev_item, next_items, blk, par):
        g = items[0][0]
        kb = kbs[par]
        gn = jnp.minimum(g + 1, NG - 1)
        n_items = len(items)
        ngr = T // 16
        piece = lambda c: (c // (TT // T)) * PPC + c % (TT // T)
        spare = lambda c: (c // (TT // T)) * PPC + TT // T
        order = [None] * NT
        for xt, pos, _ in EXTRA:
            order[pos] = xt
        use = {c: [piece(c), spare(c)] if c in order else [piece(c)] for c in range(NT)}
        rest = [c for c in range(NT) if c not in order]
        order = [c if c is not None else rest.pop(0) for c in order]
        tiles = [(u, c) for u in range(n_items) for c in order]
        stream = [(u, c, gr) for (u, c) in tiles
                  for gr in range(ngr - 1, len(use[c]) - 1, -1)]
        end = {(u, c): n + 1 for n, (u, c, _) in enumerate(stream)}
        slots = {end[tiles[0]] + DELAY - (NCARRY - i) * (ngr - 1): i for i in range(NCARRY)}
        for t in tiles[:len(tiles) - NCARRY]:
            slots[end[t] + DELAY] = t
        cuts = sorted(set(slots) | {end[(u, NT - 1)] for u in range(n_items)})
        release = [[(u, j, piece(c)) for j in range(4)] for (u, c) in tiles]
        for u in range(n_items):
            for xt, _, rel in EXTRA:
                for j in range(4):
                    release[u * NT + rel[j]].append((u, j, spare(xt)))
        spl = len(tiles) * (NT // QB) // T
        ws, sres, l, acc, probs, vres = {}, {}, {}, {}, {}, {}
        always = jnp.full((8, T), ok_ref[0], jnp.int32) != 0
        zero = opaque_zero()
        lastdep, lastbuilt, lastextra = None, [], []

        def vpu_scores(u, j, pc, dep):
            hh = 4 * items[u][1] + j
            kv = kb[pc, DH * hh:DH * (hh + 1)].reshape(DH, VK // 8, 8, T)
            qv = qb_ref[u, DH * j:DH * (j + 1)]
            if dep is not None:
                qv = jnp.concatenate(
                    [jnp.where(always[None], qv[0:1], dep[None]), qv[1:]], axis=0)
            return jnp.sum(kv * qv[:, None], axis=0).reshape(VK, T)

        def do_pv(u, c):
            p = probs.pop((u, c))
            vs = v_rows4(g, items[u][1], PT + c)
            for j in range(4):
                o = _dot(vs[j], p[:, j * T:(j + 1) * T])
                acc[(u, j)] = o + (zero if c == 0 else acc[(u, j)])
            if c == NT - 1:
                finalize(items[u], [acc[(u, j)] for j in range(4)], l[u])

        head = release[0] + release[1]
        for unit in head:
            vres[unit] = vpu_scores(*unit, None)
        hres = [vres[unit] for unit in head]
        x = 0
        for y in cuts:
            ch = stream[x:y]
            u = ch[0][0]
            _, half, q = items[u]
            if u not in ws:
                ws[u] = q_weights(g, range(4 * half, 4 * half + 4), q, base=4 * half)
            ksrc, koff = (khu, 0) if half else (ku, PT)
            rows = []
            for c in dict.fromkeys(c for (_, c, _) in ch):
                grs = [gr for (_, cc, gr) in ch if cc == c]
                r0 = (koff + c) * (T // 2) + 8 * grs[-1]
                kt = ksrc[g, r0:r0 + 8 * len(grs), :]
                rows += [kt[8 * (gr - grs[-1]):8 * (gr - grs[-1] + 1)] for gr in grs]
            for e, hr in enumerate(hres):
                if x <= e + 4 < y:
                    rows[e + 4 - x] = jnp.where(always, rows[e + 4 - x], pltpu.bitcast(
                        jnp.maximum(hr[0:8], hr[8:16]), U32))
            x = y
            lhs = jnp.concatenate(rows, axis=0)
            sc = _dot(_bf(lhs), ws[u])
            if y in slots:
                if isinstance(slots[y], int):
                    finish_carry(prev_item, slots[y])
                else:
                    do_pv(*slots[y])
            n0 = 0
            for c in dict.fromkeys(c for (_, c, _) in ch):
                cnt = sum(cc == c for (_, cc, _) in ch)
                sres.setdefault((u, c), []).append(sc[16 * n0:16 * (n0 + cnt)])
                n0 += cnt
            for (_, c, gr) in ch:
                nv = len(use[c])
                if gr != nv:
                    continue
                n = tiles.index((u, c))
                st = jnp.concatenate(sres.pop((u, c)), axis=0)
                d = blk * (len(tiles) // spl) + n // spl
                pa = (n % spl) * PPC
                pb = pa + PPC - (pa + PPC - 1 not in [spare(xt) for xt, _, _ in EXTRA])
                src = kf_ref[gn, pa:pb].reshape((pb - pa) * VK, T)
                colv = jnp.take_along_axis(
                    src, jnp.full(src.shape, d, jnp.int32), axis=1, mode="promise_in_bounds")
                kbs[1 - par][pa:pb, d] = colv.reshape(pb - pa, VK, T)
                built = colv
                if u < 2:
                    build_qb(items[n_items - 2 + u], n_items - 2 + u, n % NT)
                else:
                    build_qb(next_items[u - 2], u - 2, n % NT)
                todo = release[n]
                for e, unit in enumerate(todo):
                    if unit in head:
                        continue
                    rr = ((e * (lastdep.shape[0] // 8)) // len(todo)) ^ 1
                    dep = jnp.maximum(lastdep[rr * 8:(rr + 1) * 8, 0:T],
                                      lastbuilt[e * 8:(e + 1) * 8])
                    if e == 0:
                        for xr in lastextra:
                            dep = jnp.maximum(dep, jnp.maximum(xr[0:8], xr[8:16]))
                    vres[unit] = vpu_scores(*unit, dep)
                lastextra = [vres[unit] for unit in todo[4:]]
                parts = [jnp.concatenate([vres.pop((u, j, pc)) for j in range(4)], axis=1)
                         for pc in reversed(use[c])]
                p = jnp.exp2(jnp.concatenate([st] + parts, axis=0))
                if c == 0:
                    l[u] = jnp.sum(p.reshape(T // 8, 8, 4 * T), axis=0)
                else:
                    l[u] = jnp.sum(jnp.concatenate([l[u], p], axis=0).reshape(
                        T // 8 + 1, 8, 4 * T), axis=0)
                p = jnp.concatenate(
                    [p[16 * gg:16 * (gg + 1)] for gg in range(ngr - 1, -1, -1)], axis=0)
                if n >= len(tiles) - NCARRY:
                    cp_ref[n - (len(tiles) - NCARRY)] = p
                else:
                    probs[(u, c)] = p
                lastdep, lastbuilt = st, built
        ca_ref[...] = jnp.stack([acc[(n_items - 1, j)] for j in range(4)])
        m_ref[0] = l[n_items - 1]

    def attn_full_fast():
        nb = NT // QB

        def items(g, blk):
            return [(g, half, blk * QB + dq) for dq in range(QB) for half in range(2)]

        def items_at(b):
            return items(lax.shift_right_logical(b, nb.bit_length() - 1),
                         lax.bitwise_and(b, nb - 1))

        for u, item in enumerate(items(0, 0)[:-2]):
            for step in range(NT):
                build_qb(item, u, step)

        def outer(gp, carry):
            for par in range(2):
                g = 2 * gp + par

                def body(blk, c2, g=g, par=par):
                    prev = items_at(jnp.maximum(g * nb + blk - 1, 0))[-1]
                    nxt = items_at(jnp.minimum(g * nb + blk + 1, NG * nb - 1))
                    block_full(items(g, blk), prev, nxt, blk, par)
                    return c2
                lax.fori_loop(0, nb, body, 0)
            return carry
        lax.fori_loop(0, NG // 2, outer, 0)
        for i in range(NCARRY):
            finish_carry(items(NG - 1, nb - 1)[-1], i)

    def attn_window_fast():
        zero = opaque_zero()
        lane_grp = lax.broadcasted_iota(jnp.int32, (8, T), 1) // SQ

        def l_slot(g, u):
            return (2 * g + u // 4, slice(None), slice((u % 4) * T, (u % 4 + 1) * T))

        def qk_ops(g, b, interior):
            qg = qu[b, g]
            state = {}

            def run(u, i):
                if i == 0:
                    w = jnp.concatenate(
                        [jnp.where(lane_grp == (hh + u) % NS, qg[8 * hh:8 * (hh + 1)],
                                   jnp.zeros((8, T), U32)) for hh in range(8)], axis=0)
                    state[u] = [_bf(w), None]
                r0, r1 = WCH[i], WCH[i + 1]
                kwin = ku.at[g, pl.ds(_mul(b, T // 2), 3 * T // 2)]
                sc = _dot(_bf(kwin[(SQ * u + r0) // 2:(SQ * u + r1) // 2, :]), state[u][0])

                def post():
                    m0 = max(r0, WIN) if interior and r0 >= SQ else r0
                    m1 = min(r1, SQ) if interior and r1 <= WIN else r1
                    z = sc
                    if m1 > m0:
                        bias = wb_ref[jnp.minimum(NS * b + u, 2 * NS), m0:m1, :]
                        z = jnp.concatenate(
                            [e for e in (z[:m0 - r0], z[m0 - r0:m1 - r0] + bias, z[m1 - r0:])
                             if e.shape[0]], axis=0)
                    p = jnp.exp2(z)
                    ps = jnp.sum(p.reshape((r1 - r0) // 8, 8, T), axis=0)
                    state[u][1] = ps if i == 0 else state[u][1] + ps
                    p_ref[g, u, r0:r1, :] = p.astype(BF16)
                    if i == len(WCH) - 2:
                        m_ref[l_slot(g, u)] = state[u][1]
                return post

            return [lambda u0=u0, i=i: [run(u, i) for u in range(u0, u0 + 4)]
                    for u0 in range(0, NS, 4) for i in range(len(WCH) - 1)]

        def regroup(src, idx):
            grp = lax.broadcasted_iota(jnp.int32, src[0].shape, 1) // SQ
            src = dict(enumerate(src))
            sh = 1
            while sh < NS:
                bit = (grp & sh) != 0
                src = {i: jnp.where(bit, src[(i + sh) % NS], src[i]) for i in idx}
                sh *= 2
            return src

        def pv_ops(g, b):
            acc = [None] * 8

            def run(k, c):
                idx = range(k, NS, 2)
                parts = []
                for u in range(NS):
                    lo = c * T - SQ * u
                    r0, r1 = max(lo, 0), min(lo + T, WIN + SQ)
                    pieces = []
                    if r0 > lo:
                        pieces.append(jnp.zeros(((r0 - lo) // 2, T), U32))
                    pieces.append(pltpu.bitcast(p_ref[g, u, r0:r1, :], U32))
                    if lo + T > r1:
                        pieces.append(jnp.zeros(((lo + T - r1) // 2, T), U32))
                    parts.append(jnp.concatenate(pieces, axis=0))
                vv = vu[b + c, g]
                ps = regroup(parts, idx)
                for i in idx:
                    hh = -i % NS
                    o = _dot(_bf(vv[8 * hh:8 * (hh + 1)]), _bf(ps[i]))
                    acc[hh] = o + (zero if c == 0 else acc[hh])
                if c == 2:
                    ls = regroup([m_ref[l_slot(g, u)] for u in range(NS)], idx)
                    for i in idx:
                        hh = -i % NS
                        o = acc[hh] * _recip(jnp.sum(ls[i], axis=0, keepdims=True))
                        store_o(g, hh, b, pltpu.roll(o, T - SQ * hh, 1) if hh else o)

            return [lambda c=c, k=k: run(k, c) for c in range(3) for k in range(2)]

        def body(bb, carry):
            npc = NWP // (NT // WQ)
            for dq in range(WQ):
                b = bb * WQ + dq
                for g in range(NG):
                    i, r = divmod(dq * NG + g - 2, 3)
                    if r == 0 and 0 <= i < npc:
                        transpose_wb(bb * npc + i)
                    qk = qk_ops(g, b, dq >= PT)
                    bp = b if g else (b - 1 if dq else jnp.maximum(b - 1, 0))
                    pv = pv_ops((g - 1) % NG, bp)
                    last = dq == WQ - 1 and g == NG - 1
                    for qk_p in qk:
                        posts = qk_p()
                        for _ in range(min(2 if last else 1, len(pv))):
                            pv.pop(0)()
                        for post in posts:
                            post()
            return carry
        lax.fori_loop(0, NT // WQ, body, 0)
        for pv_p in pv_ops(NG - 1, NT - 1):
            pv_p()

    project(None, 0)
    for cp in wb_copies:
        cp.wait()

    def two_layers(it, carry):
        lax.cond(ok_ref[0] != 0, attn_window_fast, lambda: attn_max(True))
        project(0, 1)
        lax.cond(ok_ref[0] != 0, attn_full_fast, lambda: attn_max(False))
        pl.when(it == 0)(lambda: project(1, 0))
        return carry
    lax.fori_loop(0, 2, two_layers, 0)
    finish(1)


@jax.jit
def pallas_interleave_layers__sliding_block__mha_block__prompt_kernel(
    A_x: jax.Array,
    A_wqkv: jax.Array,
    A_wo: jax.Array,
    B_x: jax.Array,
    B_wqkv: jax.Array,
    B_wo: jax.Array,
):
    del B_x
    x = A_x.reshape(S, D)
    out = pl.pallas_call(
        _kernel,
        out_shape=jax.ShapeDtypeStruct((S, D), A_x.dtype),
        in_specs=[pl.BlockSpec(memory_space=pl.ANY)] * 5,
        out_specs=pl.BlockSpec(memory_space=pl.ANY),
        scratch_shapes=[
            pltpu.VMEM((S, D), BF16),
            pltpu.VMEM((3, D, D), BF16),
            pltpu.VMEM((5, D, D), BF16),
            pltpu.SemaphoreType.DMA((2 * NX + 8,)),
            pltpu.VMEM((D, S), F32),
            pltpu.VMEM((3 * D, D), BF16),
            pltpu.VMEM((5 * D, D), BF16),
            pltpu.VMEM((NT, NG, T // 2, T), U32),
            pltpu.VMEM((NG, (S + WIN) // 2, T), U32),
            pltpu.VMEM((NG, S // 2, T), U32),
            pltpu.VMEM((NT + PT, NG, T // 2, T), U32),
            pltpu.VMEM((D, S), BF16),
            pltpu.VMEM((S, 4 * T), F32),
            pltpu.VMEM((8, 8, 4 * T), F32),
            pltpu.VMEM((3, 3 * T, T), F32),
            pltpu.VMEM((2 * NS + 1, WIN + 32, T), F32),
            pltpu.VMEM((NG, 8, 3 * T, T), BF16),
            pltpu.VMEM((2 * QB, 4 * DH, 8, T), F32),
            pltpu.VMEM((NPIECE, T, VK, T), F32),
            pltpu.VMEM((NPIECE, T, VK, T), F32),
            pltpu.VMEM((NG, NPIECE, VK, T), F32),
            pltpu.VMEM((NCARRY, T, 4 * T), F32),
            pltpu.VMEM((4, DH, T), F32),
            pltpu.VMEM((4, 8, HT), F32),
            pltpu.SMEM((1,), jnp.int32),
        ],
        compiler_params=pltpu.CompilerParams(vmem_limit_bytes=100 * 1024 * 1024),
        name="interleave_attn",
    )(x, A_wqkv, A_wo, B_wqkv, B_wo)
    return out.reshape(A_x.shape)
```

```python
import math

import jax
import jax.numpy as jnp
from jax import lax
import jax.experimental.pallas as pl
import jax.experimental.pallas.tpu as pltpu

S = 2048
D = 512
H = 32
DH = 16
WIN = 256
EPS = 1e-5

T = 128
NT = S // T
NG = D // T
PT = WIN // T
NEG = -1e30
QSCALE = (DH ** -0.5) * math.log2(math.e)
TT = 512
HT = TT // 2
NX = S // TT

SMAX = 60.0
VMAX = 2.0 ** 50
VMIN = 2.0 ** -40

QB = 2
VK = 16
PPC = TT // T + 1
NPIECE = NX * PPC
XSLOT = 1
EXTRA = ((13, 13, (2, 5, 8, 11)), (9, 12, (1, 4, 7, 10)), (5, 11, (0, 3, 6, 9)))
DELAY = 9
NCARRY = 2
NS = 8
SQ = T // NS
WCH = (0, 96, 192, WIN + SQ)
WQ = 4
NWP = 5 * D // T

F32 = jnp.float32
BF16 = jnp.bfloat16
U32 = jnp.uint32


def _dot(a, b):
    return jnp.dot(a, b, preferred_element_type=F32)


def _bf(x):
    return pltpu.bitcast(x, BF16)


def _pk(x):
    return pltpu.bitcast(x.astype(BF16), U32)


def _recip(x):
    r = pl.reciprocal(x, approx=True)
    return r * (2.0 - x * r)


def _mul(a, n):
    return a * n if isinstance(a, int) else pl.multiple_of(a * n, n)


def _kernel(x_hbm, awqkv_hbm, awo_hbm, bwqkv_hbm, bwo_hbm, out_hbm,
            x_ref, wa_ref, wb2_ref, sems, xT_ref, waT_ref, wbT_ref,
            qu, ku, khu, vu, oT_ref, s_ref, m_ref, bias_ref, wb_ref,
            p_ref, qb_ref, kb0_ref, kb1_ref, kf_ref, cp_ref, ca_ref, st_ref, ok_ref):
    kbs = (kb0_ref, kb1_ref)

    def x_copy(i):
        return pltpu.make_async_copy(x_hbm.at[pl.ds(i * HT, HT)],
                                     x_ref.at[pl.ds(i * HT, HT)], sems.at[i])

    def out_copy(i):
        return pltpu.make_async_copy(x_ref.at[pl.ds(i * HT, HT)],
                                     out_hbm.at[pl.ds(i * HT, HT)], sems.at[i])

    wa_copies = [pltpu.make_async_copy(awqkv_hbm.at[:, j * D:(j + 1) * D], wa_ref.at[j],
                                       sems.at[2 * NX + j]) for j in range(3)]
    wb_src = [awo_hbm] + [bwqkv_hbm.at[:, j * D:(j + 1) * D] for j in range(3)] + [bwo_hbm]
    wb_copies = [pltpu.make_async_copy(src, wb2_ref.at[j], sems.at[2 * NX + 3 + j])
                 for j, src in enumerate(wb_src)]

    def wqkv_t(li, j):
        return waT_ref[j * D:(j + 1) * D, :] if li == 0 else wbT_ref[(j + 1) * D:(j + 2) * D, :]

    def wo_t(li):
        return wbT_ref[0:D, :] if li == 0 else wbT_ref[4 * D:5 * D, :]

    def transpose_wb(piece):
        cols = pl.ds(_mul(lax.bitwise_and(piece, NG - 1), T), T)
        w = wb2_ref[lax.shift_right_logical(piece, 2), :, cols]
        wbT_ref[pl.ds(_mul(piece, T), T), :] = w.astype(F32).T.astype(BF16)

    x_copy(0).start()
    for cp in wa_copies:
        cp.start()
    x_copy(1).start()
    x_copy(2).start()
    for g in range(NG):
        ku[g, 0:WIN // 2, :] = jnp.zeros((WIN // 2, T), U32)
    for c in range(PT):
        vu[c] = jnp.zeros((NG, T // 2, T), U32)
    row = lax.broadcasted_iota(jnp.int32, (3 * T, T), 0)
    col = lax.broadcasted_iota(jnp.int32, (3 * T, T), 1)
    band = (row > col) & (row <= col + WIN)
    for v in range(3):
        bias_ref[v] = jnp.where(band & (row >= WIN - v * T), 0.0, NEG).astype(F32)
    row = lax.broadcasted_iota(jnp.int32, (WIN + SQ, T), 0)
    col = lax.broadcasted_iota(jnp.int32, (WIN + SQ, T), 1) % SQ
    band = (row > col) & (row <= col + WIN)
    for v in range(2 * NS + 1):
        wb_ref[v, 0:WIN + SQ] = jnp.where(
            band & (row >= WIN - v * SQ), 0.0, NEG).astype(F32)
    p_ref[NG - 1] = jnp.zeros(p_ref.shape[1:], BF16)
    m_ref[...] = jnp.zeros(m_ref.shape, F32)
    cp_ref[...] = jnp.zeros(cp_ref.shape, F32)
    ca_ref[...] = jnp.zeros(ca_ref.shape, F32)
    oT_ref[...] = jnp.zeros(oT_ref.shape, BF16)

    def head_norm2(a):
        n2 = jnp.sum((a * a).reshape(H, DH, HT), axis=1)
        return jnp.max(n2.reshape(H // 8, 8, HT), axis=0)

    def residual(lo, i):
        return xT_ref[i] + _dot(wo_t(lo), oT_ref[i])

    def normalize(lo, i):
        if lo is None:
            x = x_ref[pl.ds(_mul(i, HT), HT), :].astype(F32).T
        else:
            x = residual(lo, i)
        xT_ref[i] = x
        mu = jnp.mean(x, axis=0, keepdims=True)
        xc = x - mu
        var = jnp.mean(xc * xc, axis=0, keepdims=True)
        return (xc * lax.rsqrt(var + EPS)).astype(BF16)

    def qkv(li, t, hf, xn, which):
        for w in which:
            qkv1(li, t, hf, xn, w)

    def qkv1(li, t, hf, xn, which):
        full = li == 1
        hh0 = _mul(t, TT // 2) + hf * (HT // 2)
        c0 = t * (TT // T) + hf * (HT // T)
        if which == 'k':
            kT = _dot(wqkv_t(li, 1), xn)
            st_ref[1] = jnp.maximum(st_ref[1], head_norm2(kT))
            kf = kT.T
            kk = kf.astype(BF16)
            for g in range(NG):
                ku[g, pl.ds(WIN // 2 + hh0, HT // 2), :] = _pk(kf[:, g * T:(g + 1) * T])
            if full:
                for g in range(NG):
                    khu[g, pl.ds(hh0, HT // 2), :] = _pk(
                        pltpu.roll(kf[:, g * T:(g + 1) * T], T // 2, 1))
                for c in range(HT // T):
                    cl = hf * (HT // T) + c
                    pieces = [(cl, c * T)]
                    if cl == XSLOT:
                        pieces.append((TT // T, c * T + VK))
                    for slot, r0 in pieces:
                        piece = t * PPC + slot
                        for g in range(NG):
                            kf_ref[g, piece] = kk[r0:r0 + VK, g * T:(g + 1) * T].astype(F32)
                        kp = kk[r0:r0 + VK, 0:T].astype(F32)
                        kb0_ref[piece] = jnp.stack(
                            [jnp.broadcast_to(kp[:, d:d + 1], (VK, T)) for d in range(T)])
        if which == 'q':
            q = _dot(wqkv_t(li, 0), xn) * QSCALE
            st_ref[0] = jnp.maximum(st_ref[0], head_norm2(q))
            for c in range(HT // T):
                qc = q[:, c * T:(c + 1) * T]
                if not full:
                    qc = jnp.concatenate(
                        [pltpu.roll(qc[DH * h:DH * (h + 1)], SQ * (h % NS), 1)
                         if h % NS else qc[DH * h:DH * (h + 1)] for h in range(H)], axis=0)
                for g in range(NG):
                    qu[c0 + c, g] = _pk(qc[g * T:(g + 1) * T])
        if which == 'v':
            v = _dot(wqkv_t(li, 2), xn)
            st_ref[2] = jnp.maximum(
                st_ref[2], jnp.max(jnp.abs(v).reshape(D // 8, 8, HT), axis=0))
            for c in range(HT // T):
                for g in range(NG):
                    vu[PT + c0 + c, g] = _pk(v[g * T:(g + 1) * T, c * T:(c + 1) * T])

    def project(lo, li):
        st_ref[...] = jnp.zeros(st_ref.shape, F32)
        if lo is None:
            x_copy(0).wait()
            first = normalize(None, 0)
            for j in range(3):
                wa_copies[j].wait()
                waT_ref[j * D:(j + 1) * D, :] = wa_ref[j].astype(F32).T.astype(BF16)

            def body(t, xn0):
                tn = jnp.minimum(t + 1, NX - 1)
                x_copy(2 * t + 1).wait()
                pl.when(t + 1 < NX)(lambda: x_copy(2 * tn).wait())

                @pl.when(t == 0)
                def _():
                    for i in range(3, 2 * NX):
                        x_copy(i).start()
                    for cp in wb_copies:
                        cp.start()
                xn1 = normalize(None, 2 * t + 1)
                qkv(li, t, 0, xn0, 'vqk')
                qkv(li, t, 1, xn1, 'kq')
                nxt = normalize(None, 2 * tn)
                qkv(li, t, 1, xn1, 'v')
                return nxt
            lax.fori_loop(0, NX, body, first)
        else:
            def body(t, carry):
                xns = [normalize(lo, 2 * t + hf) for hf in range(2)]
                for hf in range(2):
                    qkv(li, t, hf, xns[hf], 'kqv')
                return carry
            lax.fori_loop(0, NX, body, 0)
        qk2 = jnp.max(st_ref[0]) * jnp.max(st_ref[1])
        vm = jnp.max(st_ref[2])
        ok = (qk2 * 1.05 <= SMAX * SMAX) & (vm <= VMAX) & (vm >= VMIN)
        ok_ref[0] = ok.astype(jnp.int32)

    def finish(lo):
        def body(t, carry):
            for hf in range(4):
                i = 4 * t + hf
                x_ref[pl.ds(_mul(i, HT), HT), :] = residual(lo, i).T.astype(BF16)
                out_copy(i).start()
            return carry
        lax.fori_loop(0, S // (4 * HT), body, 0)
        for i in range(S // HT):
            out_copy(i).wait()

    def q_weights(g, heads, qi, rotated=False, base=0):
        cols = []
        for hh in heads:
            parts = []
            if hh > base:
                parts.append(jnp.zeros((8 * (hh - base), T), U32))
            slab = qu[qi, g, 8 * hh:8 * (hh + 1), :]
            if rotated and hh % NS:
                slab = pltpu.roll(slab, T - SQ * (hh % NS), 1)
            parts.append(slab)
            if hh - base < 7:
                parts.append(jnp.zeros((8 * (7 - hh + base), T), U32))
            cols.append(jnp.concatenate(parts, axis=0))
        return _bf(jnp.concatenate(cols, axis=1))

    def v_rows(g, hh, kt):
        return _bf(vu[kt, g, 8 * hh:8 * (hh + 1), :])

    def v_rows4(g, half, kt):
        vv = vu[kt, g, 32 * half:32 * (half + 1), :]
        return [_bf(vv[8 * j:8 * (j + 1)]) for j in range(4)]

    def store_o(g, hh, qi, val):
        if isinstance(qi, int):
            i, c = divmod(qi, HT // T)
        else:
            i, c = lax.shift_right_logical(qi, 1), lax.bitwise_and(qi, 1)
        oT_ref[i, pl.ds(_mul(g, T) + DH * hh, val.shape[0]), pl.ds(_mul(c, T), T)] = (
            val.astype(BF16))

    def attend_max(g, q, k0, nc, ct, bias):
        ck = ct * T
        for half in range(2):
            heads = range(4 * half, 4 * half + 4)
            w = q_weights(g, heads, q, rotated=bias is not None)

            def scores(i, m):
                sc = _dot(_bf(ku[g, pl.ds(_mul(k0 + i * ct, T // 2), ck // 2), :]), w)
                if bias is not None:
                    sc = sc + jnp.concatenate([bias[...]] * 4, axis=1)
                s_ref[pl.ds(_mul(i, ck), ck), :] = sc
                return jnp.maximum(m, jnp.max(sc.reshape(ck // 8, 8, 4 * T), axis=0))
            m = lax.fori_loop(0, nc, scores, jnp.full((8, 4 * T), -jnp.inf, F32))
            m = jnp.max(m, axis=0, keepdims=True)

            def weigh(i, carry):
                l, acc = carry
                p = jnp.exp2(s_ref[pl.ds(_mul(i, ck), ck), :] - m)
                l = l + jnp.sum(p.reshape(ck // 8, 8, 4 * T), axis=0)
                acc = list(acc)
                for j, hh in enumerate(heads):
                    for c in range(ct):
                        acc[j] = acc[j] + _dot(
                            v_rows(g, hh, k0 + i * ct + c),
                            p[c * T:(c + 1) * T, j * T:(j + 1) * T].astype(BF16))
                return l, tuple(acc)
            l, acc = lax.fori_loop(
                0, nc, weigh,
                (jnp.zeros((8, 4 * T), F32), (jnp.zeros((DH, T), F32),) * 4))
            linv = 1.0 / jnp.sum(l, axis=0, keepdims=True)
            for j, hh in enumerate(heads):
                store_o(g, hh, q, acc[j] * linv[:, j * T:(j + 1) * T])

    def attn_max(window):
        def body(b, carry):
            g = lax.shift_right_logical(b, 4)
            q = lax.bitwise_and(b, NT - 1)
            if window:
                attend_max(g, q, q, 1, 3, bias_ref.at[jnp.minimum(q, 2)])
            else:
                attend_max(g, q, PT, NT // 4, 4, None)
            return carry
        lax.fori_loop(0, NG * NT, body, 0)
        if window:
            def tr(piece, carry):
                transpose_wb(piece)
                return carry
            lax.fori_loop(0, NWP, tr, 0)

    carry_acc = [None] * 4

    def opaque_zero():
        return (jnp.full((DH, T), ok_ref[0], jnp.int32) - 1).astype(F32)

    def finalize(item, acc, l):
        g, half, q = item
        linv = _recip(jnp.sum(l, axis=0, keepdims=True))
        o = jnp.concatenate([acc[j] * linv[:, j * T:(j + 1) * T] for j in range(4)], axis=0)
        store_o(g, 4 * half, q, o)

    def finish_carry(item, i):
        vs = v_rows4(item[0], item[1], PT + NT - NCARRY + i)
        for j in range(4):
            o = _dot(vs[j], cp_ref[i, :, j * T:(j + 1) * T])
            carry_acc[j] = (ca_ref[j] if i == 0 else carry_acc[j]) + o
        if i == NCARRY - 1:
            finalize(item, carry_acc, m_ref[0])

    def build_qb(item, slot, step):
        g, half, q = item
        hh = 4 * half + step // 4
        qs = _bf(qu[q, g, 8 * hh:8 * (hh + 1), :]).astype(F32)
        qb_ref[slot, 4 * step:4 * step + 4] = jnp.stack(
            [jnp.broadcast_to(qs[r % DH:r % DH + 1, :], (8, T))
             for r in range(4 * step, 4 * step + 4)])

    def block_full(items, prev_item, next_items, blk, par):
        g = items[0][0]
        kb = kbs[par]
        gn = jnp.minimum(g + 1, NG - 1)
        n_items = len(items)
        ngr = T // 16
        piece = lambda c: (c // (TT // T)) * PPC + c % (TT // T)
        spare = lambda c: (c // (TT // T)) * PPC + TT // T
        order = [None] * NT
        for xt, pos, _ in EXTRA:
            order[pos] = xt
        use = {c: [piece(c), spare(c)] if c in order else [piece(c)] for c in range(NT)}
        rest = [c for c in range(NT) if c not in order]
        order = [c if c is not None else rest.pop(0) for c in order]
        tiles = [(u, c) for u in range(n_items) for c in order]
        stream = [(u, c, gr) for (u, c) in tiles
                  for gr in range(ngr - 1, len(use[c]) - 1, -1)]
        end = {(u, c): n + 1 for n, (u, c, _) in enumerate(stream)}
        slots = {end[tiles[0]] + DELAY - (NCARRY - i) * (ngr - 1): i for i in range(NCARRY)}
        for t in tiles[:len(tiles) - NCARRY]:
            slots[end[t] + DELAY] = t
        cuts = sorted(set(slots) | {end[(u, NT - 1)] for u in range(n_items)})
        release = [[(u, j, piece(c)) for j in range(4)] for (u, c) in tiles]
        for u in range(n_items):
            for xt, _, rel in EXTRA:
                for j in range(4):
                    release[u * NT + rel[j]].append((u, j, spare(xt)))
        spl = len(tiles) * (NT // QB) // T
        ws, sres, l, acc, probs, vres = {}, {}, {}, {}, {}, {}
        always = jnp.full((8, T), ok_ref[0], jnp.int32) != 0
        zero = opaque_zero()
        lastdep, lastbuilt, lastextra = None, [], []

        def vpu_scores(u, j, pc, dep):
            hh = 4 * items[u][1] + j
            kv = kb[pc, DH * hh:DH * (hh + 1)].reshape(DH, VK // 8, 8, T)
            qv = qb_ref[u, DH * j:DH * (j + 1)]
            if dep is not None:
                qv = jnp.concatenate(
                    [jnp.where(always[None], qv[0:1], dep[None]), qv[1:]], axis=0)
            return jnp.sum(kv * qv[:, None], axis=0).reshape(VK, T)

        def do_pv(u, c):
            p = probs.pop((u, c))
            vs = v_rows4(g, items[u][1], PT + c)
            for j in range(4):
                o = _dot(vs[j], p[:, j * T:(j + 1) * T])
                acc[(u, j)] = o + (zero if c == 0 else acc[(u, j)])
            if c == NT - 1:
                finalize(items[u], [acc[(u, j)] for j in range(4)], l[u])

        head = release[0] + release[1]
        for unit in head:
            vres[unit] = vpu_scores(*unit, None)
        hres = [vres[unit] for unit in head]
        x = 0
        for y in cuts:
            ch = stream[x:y]
            u = ch[0][0]
            _, half, q = items[u]
            if u not in ws:
                ws[u] = q_weights(g, range(4 * half, 4 * half + 4), q, base=4 * half)
            ksrc, koff = (khu, 0) if half else (ku, PT)
            rows = []
            for c in dict.fromkeys(c for (_, c, _) in ch):
                grs = [gr for (_, cc, gr) in ch if cc == c]
                r0 = (koff + c) * (T // 2) + 8 * grs[-1]
                kt = ksrc[g, r0:r0 + 8 * len(grs), :]
                rows += [kt[8 * (gr - grs[-1]):8 * (gr - grs[-1] + 1)] for gr in grs]
            for e, hr in enumerate(hres):
                if x <= e + 4 < y:
                    rows[e + 4 - x] = jnp.where(always, rows[e + 4 - x], pltpu.bitcast(
                        jnp.maximum(hr[0:8], hr[8:16]), U32))
            x = y
            lhs = jnp.concatenate(rows, axis=0)
            sc = _dot(_bf(lhs), ws[u])
            if y in slots:
                if isinstance(slots[y], int):
                    finish_carry(prev_item, slots[y])
                else:
                    do_pv(*slots[y])
            n0 = 0
            for c in dict.fromkeys(c for (_, c, _) in ch):
                cnt = sum(cc == c for (_, cc, _) in ch)
                sres.setdefault((u, c), []).append(sc[16 * n0:16 * (n0 + cnt)])
                n0 += cnt
            for (_, c, gr) in ch:
                nv = len(use[c])
                if gr != nv:
                    continue
                n = tiles.index((u, c))
                st = jnp.concatenate(sres.pop((u, c)), axis=0)
                d = blk * (len(tiles) // spl) + n // spl
                pa = (n % spl) * PPC
                pb = pa + PPC - (pa + PPC - 1 not in [spare(xt) for xt, _, _ in EXTRA])
                src = kf_ref[gn, pa:pb].reshape((pb - pa) * VK, T)
                colv = jnp.take_along_axis(
                    src, jnp.full(src.shape, d, jnp.int32), axis=1, mode="promise_in_bounds")
                kbs[1 - par][pa:pb, d] = colv.reshape(pb - pa, VK, T)
                built = colv
                if u < 2:
                    build_qb(items[n_items - 2 + u], n_items - 2 + u, n % NT)
                else:
                    build_qb(next_items[u - 2], u - 2, n % NT)
                todo = release[n]
                for e, unit in enumerate(todo):
                    if unit in head:
                        continue
                    rr = ((e * (lastdep.shape[0] // 8)) // len(todo)) ^ 1
                    dep = jnp.maximum(lastdep[rr * 8:(rr + 1) * 8, 0:T],
                                      lastbuilt[e * 8:(e + 1) * 8])
                    if e == 0:
                        for xr in lastextra:
                            dep = jnp.maximum(dep, jnp.maximum(xr[0:8], xr[8:16]))
                    vres[unit] = vpu_scores(*unit, dep)
                lastextra = [vres[unit] for unit in todo[4:]]
                parts = [jnp.concatenate([vres.pop((u, j, pc)) for j in range(4)], axis=1)
                         for pc in reversed(use[c])]
                p = jnp.exp2(jnp.concatenate([st] + parts, axis=0))
                if c == 0:
                    l[u] = jnp.sum(p.reshape(T // 8, 8, 4 * T), axis=0)
                else:
                    l[u] = jnp.sum(jnp.concatenate([l[u], p], axis=0).reshape(
                        T // 8 + 1, 8, 4 * T), axis=0)
                p = jnp.concatenate(
                    [p[16 * gg:16 * (gg + 1)] for gg in range(ngr - 1, -1, -1)], axis=0)
                if n >= len(tiles) - NCARRY:
                    cp_ref[n - (len(tiles) - NCARRY)] = p
                else:
                    probs[(u, c)] = p
                lastdep, lastbuilt = st, built
        ca_ref[...] = jnp.stack([acc[(n_items - 1, j)] for j in range(4)])
        m_ref[0] = l[n_items - 1]

    def attn_full_fast():
        nb = NT // QB

        def items(g, blk):
            return [(g, half, blk * QB + dq) for dq in range(QB) for half in range(2)]

        def items_at(b):
            return items(lax.shift_right_logical(b, nb.bit_length() - 1),
                         lax.bitwise_and(b, nb - 1))

        for u, item in enumerate(items(0, 0)[:-2]):
            for step in range(NT):
                build_qb(item, u, step)

        def outer(gp, carry):
            for par in range(2):
                g = 2 * gp + par

                def body(blk, c2, g=g, par=par):
                    prev = items_at(jnp.maximum(g * nb + blk - 1, 0))[-1]
                    nxt = items_at(jnp.minimum(g * nb + blk + 1, NG * nb - 1))
                    block_full(items(g, blk), prev, nxt, blk, par)
                    return c2
                lax.fori_loop(0, nb, body, 0)
            return carry
        lax.fori_loop(0, NG // 2, outer, 0)
        for i in range(NCARRY):
            finish_carry(items(NG - 1, nb - 1)[-1], i)

    def attn_window_fast():
        zero = opaque_zero()
        lane_grp = lax.broadcasted_iota(jnp.int32, (8, T), 1) // SQ

        def l_slot(g, u):
            return (2 * g + u // 4, slice(None), slice((u % 4) * T, (u % 4 + 1) * T))

        def qk_ops(g, b, interior):
            qg = qu[b, g]
            state = {}

            def run(u, i):
                if i == 0:
                    w = jnp.concatenate(
                        [jnp.where(lane_grp == (hh + u) % NS, qg[8 * hh:8 * (hh + 1)],
                                   jnp.zeros((8, T), U32)) for hh in range(8)], axis=0)
                    state[u] = [_bf(w), None]
                r0, r1 = WCH[i], WCH[i + 1]
                kwin = ku.at[g, pl.ds(_mul(b, T // 2), 3 * T // 2)]
                sc = _dot(_bf(kwin[(SQ * u + r0) // 2:(SQ * u + r1) // 2, :]), state[u][0])

                def post():
                    m0 = max(r0, WIN) if interior and r0 >= SQ else r0
                    m1 = min(r1, SQ) if interior and r1 <= WIN else r1
                    z = sc
                    if m1 > m0:
                        bias = wb_ref[jnp.minimum(NS * b + u, 2 * NS), m0:m1, :]
                        z = jnp.concatenate(
                            ([sc[:m0 - r0]] if m0 > r0 else [])
                            + [sc[m0 - r0:m1 - r0] + bias]
                            + ([sc[m1 - r0:]] if m1 < r1 else []), axis=0)
                    p = jnp.exp2(z)
                    ps = jnp.sum(p.reshape((r1 - r0) // 8, 8, T), axis=0)
                    state[u][1] = ps if i == 0 else state[u][1] + ps
                    p_ref[g, u, r0:r1, :] = p.astype(BF16)
                    if i == len(WCH) - 2:
                        m_ref[l_slot(g, u)] = state[u][1]
                return post

            return [lambda u0=u0, i=i: [run(u, i) for u in range(u0, u0 + 4)]
                    for u0 in range(0, NS, 4) for i in range(len(WCH) - 1)]

        def regroup(src, idx):
            grp = lax.broadcasted_iota(jnp.int32, src[0].shape, 1) // SQ
            src = dict(enumerate(src))
            sh = 1
            while sh < NS:
                bit = (grp & sh) != 0
                src = {i: jnp.where(bit, src[(i + sh) % NS], src[i]) for i in idx}
                sh *= 2
            return src

        def pv_ops(g, b):
            acc = [None] * 8

            def run(k, c):
                idx = range(k, NS, 2)
                parts = []
                for u in range(NS):
                    lo = c * T - SQ * u
                    r0, r1 = max(lo, 0), min(lo + T, WIN + SQ)
                    pieces = []
                    if r0 > lo:
                        pieces.append(jnp.zeros(((r0 - lo) // 2, T), U32))
                    pieces.append(pltpu.bitcast(p_ref[g, u, r0:r1, :], U32))
                    if lo + T > r1:
                        pieces.append(jnp.zeros(((lo + T - r1) // 2, T), U32))
                    parts.append(jnp.concatenate(pieces, axis=0))
                vv = vu[b + c, g]
                ps = regroup(parts, idx)
                for i in idx:
                    hh = -i % NS
                    o = _dot(_bf(vv[8 * hh:8 * (hh + 1)]), _bf(ps[i]))
                    acc[hh] = o + (zero if c == 0 else acc[hh])
                if c == 2:
                    ls = regroup([m_ref[l_slot(g, u)] for u in range(NS)], idx)
                    for i in idx:
                        hh = -i % NS
                        o = acc[hh] * _recip(jnp.sum(ls[i], axis=0, keepdims=True))
                        store_o(g, hh, b, pltpu.roll(o, T - SQ * hh, 1) if hh else o)

            return [lambda c=c, k=k: run(k, c) for c in range(3) for k in range(2)]

        def body(bb, carry):
            nb = NT // WQ
            npc = NWP // nb
            for dq in range(WQ):
                b = bb + dq * nb
                for g in range(NG):
                    i, r = divmod(dq * NG + g - 2, 3)
                    if r == 0 and 0 <= i < npc:
                        transpose_wb(bb * npc + i)
                    qk = qk_ops(g, b, dq > 0)
                    bp = b if g else (b - nb if dq else jnp.maximum(bb - 1, 0) + NT - nb)
                    pv = pv_ops((g - 1) % NG, bp)
                    last = dq == WQ - 1 and g == NG - 1
                    for qk_p in qk:
                        posts = qk_p()
                        for _ in range(min(2 if last else 1, len(pv))):
                            pv.pop(0)()
                        for post in posts:
                            post()
            return carry
        lax.fori_loop(0, NT // WQ, body, 0)
        for pv_p in pv_ops(NG - 1, NT - 1):
            pv_p()

    project(None, 0)
    for cp in wb_copies:
        cp.wait()

    def two_layers(it, carry):
        lax.cond(ok_ref[0] != 0, attn_window_fast, lambda: attn_max(True))
        project(0, 1)
        lax.cond(ok_ref[0] != 0, attn_full_fast, lambda: attn_max(False))
        pl.when(it == 0)(lambda: project(1, 0))
        return carry
    lax.fori_loop(0, 2, two_layers, 0)
    finish(1)


@jax.jit
def pallas_interleave_layers__sliding_block__mha_block__prompt_kernel(
    A_x: jax.Array,
    A_wqkv: jax.Array,
    A_wo: jax.Array,
    B_x: jax.Array,
    B_wqkv: jax.Array,
    B_wo: jax.Array,
):
    del B_x
    x = A_x.reshape(S, D)
    out = pl.pallas_call(
        _kernel,
        out_shape=jax.ShapeDtypeStruct((S, D), A_x.dtype),
        in_specs=[pl.BlockSpec(memory_space=pl.ANY)] * 5,
        out_specs=pl.BlockSpec(memory_space=pl.ANY),
        scratch_shapes=[
            pltpu.VMEM((S, D), BF16),
            pltpu.VMEM((3, D, D), BF16),
            pltpu.VMEM((5, D, D), BF16),
            pltpu.SemaphoreType.DMA((2 * NX + 8,)),
            pltpu.VMEM((2 * NX, D, HT), F32),
            pltpu.VMEM((3 * D, D), BF16),
            pltpu.VMEM((5 * D, D), BF16),
            pltpu.VMEM((NT, NG, T // 2, T), U32),
            pltpu.VMEM((NG, (S + WIN) // 2, T), U32),
            pltpu.VMEM((NG, S // 2, T), U32),
            pltpu.VMEM((NT + PT, NG, T // 2, T), U32),
            pltpu.VMEM((2 * NX, D, HT), BF16),
            pltpu.VMEM((S, 4 * T), F32),
            pltpu.VMEM((8, 8, 4 * T), F32),
            pltpu.VMEM((3, 3 * T, T), F32),
            pltpu.VMEM((2 * NS + 1, WIN + 32, T), F32),
            pltpu.VMEM((NG, 8, 3 * T, T), BF16),
            pltpu.VMEM((2 * QB, 4 * DH, 8, T), F32),
            pltpu.VMEM((NPIECE, T, VK, T), F32),
            pltpu.VMEM((NPIECE, T, VK, T), F32),
            pltpu.VMEM((NG, NPIECE, VK, T), F32),
            pltpu.VMEM((NCARRY, T, 4 * T), F32),
            pltpu.VMEM((4, DH, T), F32),
            pltpu.VMEM((4, 8, HT), F32),
            pltpu.SMEM((1,), jnp.int32),
        ],
        compiler_params=pltpu.CompilerParams(vmem_limit_bytes=100 * 1024 * 1024),
        name="interleave_attn",
    )(x, A_wqkv, A_wo, B_wqkv, B_wo)
    return out.reshape(A_x.shape)
```
